```python
import os as _os
_os.environ.setdefault("JAX_PLATFORMS", "cpu")
import jax
import jax.numpy as jnp

def _softmax(x, axis=-1):
    return jax.nn.softmax(x, axis=axis)
def _gelu(x):
    return jax.nn.gelu(x, approximate=True)
def _silu(x):
    return jax.nn.silu(x)
def _sigmoid(x):
    return jax.nn.sigmoid(x)
def _layernorm(x, axis=-1, eps=1e-5):
    m = jnp.mean(x, axis=axis, keepdims=True)
    v = jnp.var(x, axis=axis, keepdims=True)
    return (x - m) / jnp.sqrt(v + eps)
def _scatter_add(tgt, idx, src, axis=0):
    return tgt.at[idx].add(src)
def _segment_sum(src, seg, n):
    return jax.ops.segment_sum(src, seg, n)
class _Rng:
    def __init__(self, key):
        self._k = key
    def _next(self):
        self._k, sub = jax.random.split(self._k)
        return sub
    def normal(self, shape):
        return jax.random.normal(self._next(), shape, dtype=jnp.bfloat16)
    def randint(self, lo, hi, shape):
        return jax.random.randint(self._next(), shape, lo, hi, dtype=jnp.int32)
    def uniform(self, shape, lo=0.0, hi=1.0):
        return jax.random.uniform(self._next(), shape, jnp.bfloat16, lo, hi)
    def permutation(self, n):
        return jax.random.permutation(self._next(), n)


kernel_name = 'gated_mix__softmax_full_mha__dense_activation_relu__prompt'

def setup_inputs():
    _rng = _Rng(jax.random.key(int.from_bytes(__import__("os").urandom(4), "little")))
    _w = (lambda a: (lambda t: t.astype(jnp.bfloat16) if jnp.issubdtype(t.dtype, jnp.floating) else t)(jnp.asarray(a)))
    def _A_setup():
        B, S, D = 1, 2048, 640
        return {
            "x": _w((lambda *s: _rng.normal(s) * 0.05)(B, S, D)),
            "wqkv": _w((lambda *s: _rng.normal(s) * 0.8)(D, 3 * D)),
            "wo": _w((lambda *s: _rng.normal(s) * 0.05)(D, D)),
        }
    _A_in = _A_setup()

    def _B_setup():
        B, S, D, Dff = 1, 2048, 640, 1536
        return {
            "x": _w((lambda *s: _rng.normal(s) * 0.05)(B, S, D)),
            "w1": _w((lambda *s: _rng.normal(s) * 0.05)(D, Dff)),
            "w2": _w((lambda *s: _rng.normal(s) * 0.05)(Dff, D)),
        }
    _B_in = _B_setup()

    return {
        "A_x": _A_in["x"],
        "A_wqkv": _A_in["wqkv"],
        "A_wo": _A_in["wo"],
        "B_x": _B_in["x"],
        "B_w1": _B_in["w1"],
        "B_w2": _B_in["w2"],
        "gate_w": _w((lambda *s: _rng.normal(s) * 0.05)(640) * 16.0),
    }

def reference(A_x, A_wqkv, A_wo, B_x, B_w1, B_w2, gate_w):
    def _A_ref(x, wqkv, wo):
        B, S, D = x.shape
        H = 32; Dh = D // H
        qkv = (lambda x, *d: x.transpose(*d))((x @ wqkv).reshape(B, S, 3, H, Dh), 2, 0, 3, 1, 4)
        q, k, v = qkv[0], qkv[1], qkv[2]
        scale = Dh ** -0.5
        scores = jnp.einsum("bhqd,bhkd->bhqk", q, k) * scale
        p = _softmax(scores, axis=-1)
        o = jnp.einsum("bhqk,bhkd->bhqd", p, v)
        return (lambda x, *d: x.transpose(*d))(o, 0, 2, 1, 3).reshape(B, S, D) @ wo

    def _B_ref(x, w1, w2):
        h = jnp.einsum("bsd,df->bsf", x, w1)
        zero = jnp.zeros_like(h)
        h = jnp.maximum(h, zero)
        return jnp.einsum("bsf,fd->bsd", h, w2)

    x = A_x
    g = _sigmoid((x * gate_w).sum(-1, keepdims=True))
    a = _A_ref(x, A_wqkv, A_wo)
    b = _B_ref(x, B_w1, B_w2)
    return g * a + (1 - g) * b
```

```python
import functools
import math
import jax
import jax.numpy as jnp
from jax import lax
import jax.experimental.pallas as pl
import jax.experimental.pallas.tpu as pltpu

S, D, H, DH, DFF = 2048, 640, 32, 20, 1536
HP = 24
HPS = 6
NSLAB = 6
SLABW = HPS * DH
QROWS = 736
F32 = jnp.float32
BF16 = jnp.bfloat16


def make_kernel(TQ=512, KC=256, RB=512):
    NQ = S // TQ
    NSTEP = H * NQ
    NKC = S // KC
    C = (DH ** -0.5) * math.log2(math.e)

    def kernel(x_ref, wqkv_ref, wo_ref, w1_ref, w2_ref, gw_ref, out_ref,
               wks_ref, wqvt_ref, wop_ref, k_ref, qt_ref, vt_ref, ot_ref, s0_ref, s1_ref, m0_ref, m1_ref):
        lane = lax.broadcasted_iota(jnp.int32, (D, 128), 1)
        for j in range(NSLAB):
            nvalid = min(SLABW, D - SLABW * j)
            w = wqkv_ref[:, D + SLABW * j: D + SLABW * j + 128]
            wks_ref[:, 128 * j:128 * (j + 1)] = jnp.where(lane < nvalid, w, jnp.zeros_like(w))
        wqvt_ref[0:D, :] = wqkv_ref[:, 0:D].astype(F32).T
        wvt = wqkv_ref[:, 2 * D:3 * D].astype(F32).T
        wqvt_ref[D:, :] = jnp.zeros((H * HP, D), F32)
        wop_ref[...] = jnp.zeros((H * HP, D), F32)
        wo = wo_ref[...].astype(F32)
        for h in range(H):
            wqvt_ref[D + HP * h: D + HP * h + DH, :] = wvt[DH * h: DH * (h + 1), :]
            wop_ref[HP * h: HP * h + DH, :] = wo[DH * h: DH * (h + 1), :]
        qt_ref[D:, :] = jnp.zeros((QROWS - D, S), F32)

        row = lax.broadcasted_iota(jnp.int32, (H * HP, RB), 0)
        ones_row = (row % HP) == DH
        def proj(i, c):
            r0 = pl.multiple_of(i * RB, RB)
            xb = x_ref[pl.ds(r0, RB), :]
            ks = jnp.dot(xb, wks_ref[...], preferred_element_type=F32)
            for j in range(NSLAB):
                k_ref[j, pl.ds(r0, RB), :] = ks[:, 128 * j:128 * (j + 1)].astype(BF16)
            qv = lax.dot_general(wqvt_ref[...].astype(BF16), xb, (((1,), (1,)), ((), ())),
                                 preferred_element_type=F32)
            qt_ref[0:D, pl.ds(r0, RB)] = qv[0:D] * C
            vt_ref[:, pl.ds(r0, RB)] = jnp.where(ones_row, 1.0, qv[D:])
            return c
        lax.fori_loop(0, S // RB, proj, 0)

        qrow = lax.broadcasted_iota(jnp.int32, (128, TQ), 0)

        def get_qz(t):
            h = t // NQ
            qi = t % NQ
            j = h // HPS
            lo = (h % HPS) * DH
            q = qt_ref[pl.ds(pl.multiple_of(j * SLABW, 8), 128), pl.ds(pl.multiple_of(qi * TQ, TQ), TQ)]
            qz = jnp.where((qrow >= lo) & (qrow < lo + DH), q, 0.0).astype(BF16)
            return qz, j

        def stage(ta, sa_ref, ma_ref, tb, sb_ref, mb_ref):
            if ta is not None:
                qz, j = get_qz(ta)
                m8 = jnp.full((8, TQ), -jnp.inf, F32)
            if tb is not None:
                hb = tb // NQ
                qb = tb % NQ
                mb = mb_ref[...]
                acc = jnp.zeros((HP, TQ), F32)
                vrow = pl.multiple_of(hb * HP, 8)
            for c in range(NKC):
                if ta is not None:
                    s = jnp.dot(k_ref[j, c * KC:(c + 1) * KC, :], qz, preferred_element_type=F32)
                    sa_ref[c * KC:(c + 1) * KC, :] = s
                    m8 = jnp.maximum(m8, jnp.max(s.reshape(KC // 8, 8, TQ), axis=0))
                if tb is not None:
                    p = jnp.exp2(sb_ref[c * KC:(c + 1) * KC, :] - mb)
                    acc = acc + jnp.dot(vt_ref[pl.ds(vrow, HP), c * KC:(c + 1) * KC], p,
                                        preferred_element_type=F32)
            if ta is not None:
                ma_ref[...] = jnp.max(m8, axis=0, keepdims=True)
            if tb is not None:
                l = acc[DH:DH + 1, :]
                ot_ref[pl.ds(vrow, HP), pl.ds(pl.multiple_of(qb * TQ, TQ), TQ)] = acc / l

        stage(0, s0_ref, m0_ref, None, None, None)

        def body(u, c):
            t = 2 * u
            stage(t + 1, s1_ref, m1_ref, t, s0_ref, m0_ref)
            tn = jnp.minimum(t + 2, NSTEP - 1)
            stage(tn, s0_ref, m0_ref, t + 1, s1_ref, m1_ref)
            return c
        lax.fori_loop(0, NSTEP // 2, body, 0)

        gw = gw_ref[...].astype(F32)
        def fin(i, c):
            r0 = pl.multiple_of(i * RB, RB)
            xb = x_ref[pl.ds(r0, RB), :]
            ot = ot_ref[:, pl.ds(r0, RB)]
            a = lax.dot_general(ot.astype(BF16), wop_ref[...].astype(BF16), (((0,), (0,)), ((), ())),
                                preferred_element_type=F32)
            h1 = jnp.maximum(jnp.dot(xb, w1_ref[...], preferred_element_type=F32), 0.0).astype(BF16)
            b = jnp.dot(h1, w2_ref[...], preferred_element_type=F32)
            logit = jnp.sum(xb.astype(F32) * gw, axis=-1, keepdims=True)
            g = jax.nn.sigmoid(logit)
            out_ref[pl.ds(r0, RB), :] = (g * a + (1.0 - g) * b).astype(out_ref.dtype)
            return c
        lax.fori_loop(0, S // RB, fin, 0)

    scratch = [
        pltpu.VMEM((D, NSLAB * 128), BF16),
        pltpu.VMEM((D + H * HP, D), F32),
        pltpu.VMEM((H * HP, D), F32),
        pltpu.VMEM((NSLAB, S, 128), BF16),
        pltpu.VMEM((QROWS, S), F32),
        pltpu.VMEM((H * HP, S), F32),
        pltpu.VMEM((H * HP, S), F32),
        pltpu.VMEM((S, TQ), F32),
        pltpu.VMEM((S, TQ), F32),
        pltpu.VMEM((1, TQ), F32),
        pltpu.VMEM((1, TQ), F32),
    ]

    @jax.jit
    def f(A_x, A_wqkv, A_wo, B_x, B_w1, B_w2, gate_w):
        x = A_x.reshape(S, D)
        gw = gate_w.reshape(1, D)
        out = pl.pallas_call(
            kernel,
            out_shape=jax.ShapeDtypeStruct((S, D), BF16),
            scratch_shapes=scratch,
            compiler_params=pltpu.CompilerParams(vmem_limit_bytes=110 * 1024 * 1024),
        )(x, A_wqkv, A_wo, B_w1, B_w2, gw)
        return out.reshape(1, S, D)
    return f


_impl = make_kernel(TQ=512, KC=256)


@jax.jit
def pallas_gated_mix__softmax_full_mha__dense_activation_relu__prompt_kernel(
    A_x: jax.Array,
    A_wqkv: jax.Array,
    A_wo: jax.Array,
    B_x: jax.Array,
    B_w1: jax.Array,
    B_w2: jax.Array,
    gate_w: jax.Array,
):
    return _impl(A_x, A_wqkv, A_wo, B_x, B_w1, B_w2, gate_w)
```

```python
import math
import jax
import jax.numpy as jnp
from jax import lax
import jax.experimental.pallas as pl
import jax.experimental.pallas.tpu as pltpu

S, D, H, DH, DFF = 2048, 640, 32, 20, 1536
HP = 24
HPS = 6
NSLAB = 6
SLABW = HPS * DH
F32 = jnp.float32
BF16 = jnp.bfloat16


def pk(x):
    return pltpu.bitcast(x, F32)


def upk(x):
    return pltpu.bitcast(x, BF16)


def zds(z, off, n):
    if isinstance(z, int):
        return pl.ds(z + off, n)
    return pl.ds(pl.multiple_of(z * 8 + off, 8), n)


NT = (((1,), (1,)), ((), ()))
TN = (((0,), (0,)), ((), ()))


def make_kernel(TQ=512, KC=128, PK=16, FORCE_FB=0, NP=4, NG=2, TIE=0, QBM=0):
    RB = TQ
    NB = S // RB
    NQ = S // TQ
    NSTEP = H * NQ
    NKC = S // KC
    NPER = -(-NKC // NP)
    HK = KC // 2
    KM = KC - PK
    C = (DH ** -0.5) * math.log2(math.e)
    U = 2 * NQ
    NIT = NSTEP // U
    DPS = DH // NQ

    def kernel(x_hbm, wqkv_hbm, wo_hbm, w1_hbm, w2_hbm, gw_ref, out_hbm,
               x_ref, wqkv_ref, wo_ref, w1_ref, w2_ref, out_ref,
               wks_ref, wqvt_ref, k_ref, qt_ref, vt_ref, ot_ref, bm_ref, g_ref,
               qb_ref, kb0_ref, kb1_ref, p0, p1, p2, p3,
               sem_in, sem_x, sem_out):
        kbbuf = (kb0_ref, kb1_ref)
        pbuf = (p0, p1, p2, p3)

        def wq_cp(c0, c1, n):
            return pltpu.make_async_copy(wqkv_hbm.at[:, c0:c1], wqkv_ref.at[:, c0:c1], sem_in.at[n])
        cp_wk = wq_cp(D, D + 768, 0)
        cp_wq = wq_cp(0, D, 1)
        cp_wv = wq_cp(D + 768, 3 * D, 2)
        cp_x = [pltpu.make_async_copy(x_hbm.at[i * RB:(i + 1) * RB], x_ref.at[i * RB:(i + 1) * RB], sem_x.at[i])
                for i in range(NB)]
        cp_w = [pltpu.make_async_copy(a, b, sem_in.at[3 + n])
                for n, (a, b) in enumerate(((w1_hbm, w1_ref), (w2_hbm, w2_ref), (wo_hbm, wo_ref)))]
        cp_wk.start()
        cp_x[0].start()
        for pb in pbuf:
            pb[NPER * HK:2 * NPER * HK, :] = jnp.zeros((NPER * HK, TQ), F32)
        kb1_ref[0:8, :] = jnp.zeros((8, 128), F32)
        for i in range(NQ):
            qt_ref[NSLAB - 1, i, 40:120] = jnp.zeros((80, TQ), F32)

        cp_wk.wait()
        for c in cp_x[1:] + [cp_wq, cp_wv]:
            c.start()
        lane = lax.broadcasted_iota(jnp.int32, (D, 128), 1)
        for j in range(NSLAB):
            nvalid = min(SLABW, D - SLABW * j)
            w = wqkv_ref[:, D + SLABW * j: D + SLABW * j + 128]
            wks_ref[:, 128 * j:128 * (j + 1)] = jnp.where(lane < nvalid, w, jnp.zeros_like(w))

        klane = lax.broadcasted_iota(jnp.int32, (RB, 128), 1)
        kones = (klane >= SLABW) & (klane < SLABW + HPS)
        g8r = lax.broadcasted_iota(jnp.int32, (8, 128), 0)
        g8c = lax.broadcasted_iota(jnp.int32, (8, 128), 1)
        g8 = jnp.where((g8c >= g8r * DH) & (g8c < g8r * DH + DH) & (g8r < HPS), 1.0, 0.0).astype(F32)
        r8 = lax.broadcasted_iota(jnp.int32, (8, RB), 0)

        kn = [None] * NSLAB
        for i in range(NB):
            if i == 0:
                cp_x[0].wait()
            if i == 1:
                for c in cp_x[1:] + [cp_wq, cp_wv]:
                    c.wait()
                cp_w[0].start()
                cp_w[1].start()
            xb = x_ref[i * RB:(i + 1) * RB, :]
            ks = jnp.dot(xb, wks_ref[...], preferred_element_type=F32)
            for j in range(NSLAB):
                kj = ks[:, 128 * j:128 * (j + 1)]
                n2 = lax.dot_general(g8, kj * kj, NT, preferred_element_type=F32)
                kn[j] = n2 if kn[j] is None else jnp.maximum(kn[j], n2)
                k_ref[j, i * (RB // 2):(i + 1) * (RB // 2), :] = pk(jnp.where(kones, 1.0, kj).astype(BF16))
            if i == 1:
                wqvt_ref[0:D, :] = wqkv_ref[:, 0:D].astype(F32).T.astype(BF16)
            if i == 2:
                wqvt_ref[D:, :] = wqkv_ref[:, 2 * D:3 * D].astype(F32).T.astype(BF16)
        kmax = jnp.max(jnp.concatenate(kn, axis=0), axis=1, keepdims=True)

        g48r = lax.broadcasted_iota(jnp.int32, (8 * NSLAB, D), 0)
        g48c = lax.broadcasted_iota(jnp.int32, (8 * NSLAB, D), 1)
        g48h = (g48r // 8) * HPS + (g48r % 8)
        g48 = jnp.where((g48c >= g48h * DH) & (g48c < g48h * DH + DH) & (g48r % 8 < HPS), 1.0, 0.0).astype(F32)

        def prep_qb(i):
            for j in range(NSLAB):
                qj = qt_ref[j, i]
                for hh in range(j * HPS, min(H, (j + 1) * HPS)):
                    i6 = hh - j * HPS
                    for d in range(DH + 1):
                        r = i6 * DH + d if d < DH else SLABW + i6
                        rr = (hh * (DH + 1) + d) * 8
                        qb_ref[i, rr:rr + 8, :] = jnp.broadcast_to(qj[r:r + 1], (8, TQ))

        for i in range(NB):
            xb = x_ref[i * RB:(i + 1) * RB, :]
            cs = slice(i * RB, (i + 1) * RB)
            q = lax.dot_general(wqvt_ref[0:D, :], xb, NT, preferred_element_type=F32)
            q = (q * C).astype(BF16).astype(F32)
            qn = jnp.dot(g48, q * q, preferred_element_type=F32)
            nub = (-(jnp.sqrt(qn * kmax) * 1.03)).astype(BF16).astype(F32)
            for j in range(NSLAB):
                nv = min(SLABW, D - SLABW * j)
                qt_ref[j, i, 0:nv] = q[SLABW * j:SLABW * j + nv]
                qt_ref[j, i, SLABW:128] = nub[8 * j:8 * j + 8]

        def prep_kb(h, c, par, z, ds_):
            j = h // HPS
            lo = (h % HPS) * DH
            k = upk(k_ref[j, c * HK + KM // 2:(c + 1) * HK, :]).astype(F32)
            k = pltpu.roll(k, (128 - lo) % 128, 1)
            for d in ds_:
                kbbuf[par][zds(z, (d * NKC + c) * PK, PK), :] = jnp.broadcast_to(k[:, d:d + 1], (PK, 128))

        cp_w[2].start()
        cp_w[0].wait()
        cp_w[1].wait()
        gw = gw_ref[...].astype(F32)
        if PK:
            for c in range(NKC):
                prep_kb(0, c, 0, 0, range(DH))

        def vffn(i, c):
            r0 = pl.multiple_of(i * RB, RB)
            cs = pl.ds(r0, RB)
            xb = x_ref[cs, :]
            if PK:
                prep_qb(i)
            h1 = jnp.maximum(jnp.dot(xb, w1_ref[...], preferred_element_type=F32), 0.0).astype(BF16)
            b = jnp.dot(h1, w2_ref[...], preferred_element_type=F32)
            logit = jnp.sum(xb.astype(F32) * gw, axis=-1, keepdims=True)
            g = jax.nn.sigmoid(logit)
            bm_ref[cs, :] = (1.0 - g) * b
            g_ref[cs, :] = jnp.broadcast_to(g, (RB, 128))
            v = lax.dot_general(wqvt_ref[D:, :], xb, NT, preferred_element_type=F32)
            for p in range(H // 2):
                g = v[40 * p:40 * p + 40]
                mid = g[16:24]
                vt_ref[48 * p:48 * p + 16, cs] = g[0:16]
                vt_ref[48 * p + 16:48 * p + 24, cs] = jnp.where(r8 < 4, mid, jnp.where(r8 == 4, 1.0, 0.0))
                vt_ref[48 * p + 24:48 * p + 32, cs] = jnp.where(r8 >= 4, mid, jnp.where(r8 == 0, 1.0, 0.0))
                vt_ref[48 * p + 32:48 * p + 48, cs] = g[24:40]
            return c
        lax.fori_loop(0, NB, vffn, 0)

        qrow = lax.broadcasted_iota(jnp.int32, (128, TQ), 0)
        lastacc = [None]

        def stage(h, qi, cur, par, prev, nxt_head, slot, z, z2, do_a=True):
            hp, qp, orow = prev
            vrow = pl.multiple_of(hp * HP, 8)
            acc = None
            wbase = (cur % 2) * NPER * HK
            rbase = ((cur + 1) % 2) * NPER * HK
            if do_a:
                ztrue = z2 == 0
                j = h // HPS
                i6 = h % HPS
                lo = i6 * DH
                qbase = h * ((DH + 1) * 8)
                keep = ((qrow >= lo) & (qrow < lo + DH)) | (qrow == SLABW + i6)
                qz = jnp.where(keep, qt_ref[j, qi], 0.0).astype(BF16)
            for c in range(NKC):
                vt = vt_ref[pl.ds(vrow, HP), c * KC:(c + 1) * KC]
                if do_a and TIE and PK and par == 0 and c % TIE == TIE - 1:
                    t1 = kbbuf[1][zds(z2, 0, 8), :]
                    vt = jnp.concatenate([jnp.where(ztrue, vt[0:8], t1), vt[8:]], axis=0)
                pw = pbuf[c % NP][zds(z2, rbase + (c // NP) * HK, HK), :]
                d = jnp.dot(vt, upk(pw), preferred_element_type=F32)
                if acc is None:
                    acc = d if lastacc[0] is None else jnp.where(ztrue, d, lastacc[0])
                else:
                    acc = acc + d
                if not do_a:
                    continue
                s = jnp.dot(upk(k_ref[j, c * HK:c * HK + KM // 2, :]), qz, preferred_element_type=F32)
                pbuf[c % NP][zds(z, wbase + (c // NP) * HK, KM // 2), :] = pk(jnp.exp2(s).astype(BF16))
                if PK:
                    GW = TQ // NG
                    tprev = None
                    for g in range(NG):
                        def ldq(dd):
                            v = qb_ref[qi, pl.ds(pl.multiple_of(qbase + 8 * dd, 8), 8), g * GW:(g + 1) * GW]
                            return jnp.concatenate([v] * (PK // 8), axis=0)
                        t = ldq(DH)
                        if tprev is not None:
                            t = jnp.where(ztrue, t, tprev)
                        for dd in range(DH):
                            kb = kbbuf[par][zds(z2, (dd * NKC + c) * PK, PK), :]
                            kb = jnp.concatenate([kb] * (GW // 128), axis=1)
                            t = t + kb * ldq(dd)
                        pbuf[c % NP][zds(z, wbase + (c // NP) * HK + KM // 2, PK // 2), g * GW:(g + 1) * GW] = pk(
                            jnp.exp2(t).astype(BF16))
                        tprev = t
                    dsl = (range(qi * DPS, (qi + 1) * DPS) if par == 0
                           else [range(0), range(0, 7), range(7, 14), range(14, 20)][qi])
                    if len(dsl):
                        prep_kb(nxt_head, c, 1 - par, z, dsl)
            ot_ref[pl.ds(pl.multiple_of(orow, 8), HP), qp * TQ:(qp + 1) * TQ] = acc
            lastacc[0] = acc

        def body(u, c):
            z = lax.shift_right_logical(u, 8)
            z2 = lax.shift_right_logical(u, 9)
            slot = u % 2
            lastacc[0] = None
            for i in range(U):
                h = 2 * u + i // NQ
                qi = i % NQ
                if i == 0:
                    hp = jnp.maximum(2 * u - 1, 0)
                    prev = (hp, NQ - 1, jnp.where(u == 0, H * HP, hp * HP))
                else:
                    hp = 2 * u + (i - 1) // NQ
                    prev = (hp, (i - 1) % NQ, hp * HP)
                nxt_head = jnp.minimum(h + 1, H - 1)
                stage(h, qi, i, (i // NQ) % 2, prev, nxt_head, slot, z, z2)
            return c
        lax.fori_loop(0, NIT, body, 0)
        lastacc[0] = None
        stage(0, 0, 0, 0, (H - 1, NQ - 1, (H - 1) * HP), None, 0, 0, 0, do_a=False)

        r8s = lax.broadcasted_iota(jnp.int32, (8, S), 0)
        bad = jnp.zeros((8, S), F32)
        for p in range(H // 2):
            le = ot_ref[48 * p + 16:48 * p + 24, :]
            lo_ = ot_ref[48 * p + 24:48 * p + 32, :]
            l = jnp.where(r8s == 4, le, jnp.where(r8s == 0, lo_, 1.0))
            ok = (l >= 2.0 ** -60) & (l <= 4096.0)
            bad = jnp.maximum(bad, jnp.where(ok, 0.0, 1.0))
        nbad = jnp.max(jnp.max(bad, axis=1, keepdims=True), axis=0, keepdims=True)[0, 0]
        if FORCE_FB:
            nbad = nbad + 1.0


        @pl.when(nbad > 0.0)
        def _():
            def fb(t, c):
                h = t // NQ
                qi = t % NQ
                j = h // HPS
                lo = (h % HPS) * DH
                qz = jnp.where((qrow >= lo) & (qrow < lo + DH), qt_ref[j, qi], 0.0).astype(BF16)
                s = jnp.dot(upk(k_ref[j]), qz, preferred_element_type=F32)
                m = jnp.max(s, axis=0, keepdims=True)
                p = jnp.exp2(s - m).astype(BF16)
                vrow = pl.multiple_of(h * HP, 8)
                acc = jnp.dot(vt_ref[pl.ds(vrow, HP), :], p, preferred_element_type=F32)
                ot_ref[pl.ds(vrow, HP), pl.ds(pl.multiple_of(qi * TQ, TQ), TQ)] = acc
                return c
            lax.fori_loop(0, NSTEP, fb, 0)

        cp_w[2].wait()

        def out_cp(i):
            r0 = pl.multiple_of(i * RB, RB)
            return pltpu.make_async_copy(out_ref.at[pl.ds(r0, RB)], out_hbm.at[pl.ds(r0, RB)], sem_out.at[i])

        def fin(i, c):
            r0 = pl.multiple_of(i * RB, RB)
            parts = []
            for p in range(H // 2):
                e = ot_ref[48 * p:48 * p + 24, pl.ds(r0, RB)]
                o = ot_ref[48 * p + 24:48 * p + 48, pl.ds(r0, RB)]
                e = e * (1.0 / e[DH:DH + 1])
                o = o * (1.0 / o[0:1])
                parts += [e[0:16], jnp.where(r8 < 4, e[16:24], o[0:8]), o[8:24]]
            ot = jnp.concatenate(parts, axis=0).astype(BF16)
            a = lax.dot_general(ot, wo_ref[...], TN, preferred_element_type=F32)
            g = jnp.concatenate([g_ref[pl.ds(r0, RB), :]] * (D // 128), axis=1)
            out_ref[pl.ds(r0, RB), :] = (g * a + bm_ref[pl.ds(r0, RB), :]).astype(out_ref.dtype)
            out_cp(i).start()
            return c
        lax.fori_loop(0, NB, fin, 0)
        for i in range(NB):
            out_cp(i).wait()

    PKP = max(PK, 8)
    scratch = [
        pltpu.VMEM((S, D), BF16),
        pltpu.VMEM((D, 3 * D), BF16),
        pltpu.VMEM((D, D), BF16),
        pltpu.VMEM((D, DFF), BF16),
        pltpu.VMEM((DFF, D), BF16),
        pltpu.VMEM((S, D), BF16),
        pltpu.VMEM((D, NSLAB * 128), BF16),
        pltpu.VMEM((2 * D, D), BF16),
        pltpu.VMEM((NSLAB, S // 2, 128), F32),
        pltpu.VMEM((NSLAB, NQ, 128, TQ), F32),
        pltpu.VMEM((H * HP, S), F32),
        pltpu.VMEM((H * HP + HP, S), F32),
        pltpu.VMEM((S, D), F32),
        pltpu.VMEM((S, 128), F32),
        pltpu.VMEM((NQ, H * (DH + 1) * 8, TQ), F32),
        pltpu.VMEM((DH * NKC * PKP, 128), F32),
        pltpu.VMEM((DH * NKC * PKP, 128), F32),
    ] + [pltpu.VMEM((2 * NPER * HK, TQ), F32)] * NP + [
        pltpu.SemaphoreType.DMA((6,)),
        pltpu.SemaphoreType.DMA((NB,)),
        pltpu.SemaphoreType.DMA((NB,)),
    ]
    anyspec = pl.BlockSpec(memory_space=pl.ANY)

    @jax.jit
    def f(A_x, A_wqkv, A_wo, B_x, B_w1, B_w2, gate_w):
        x = A_x.reshape(S, D)
        gw = gate_w.reshape(1, D)
        out = pl.pallas_call(
            kernel,
            out_shape=jax.ShapeDtypeStruct((S, D), BF16),
            in_specs=[anyspec] * 5 + [pl.BlockSpec(memory_space=pltpu.VMEM)],
            out_specs=anyspec,
            scratch_shapes=scratch,
            compiler_params=pltpu.CompilerParams(vmem_limit_bytes=120 * 1024 * 1024),
        )(x, A_wqkv, A_wo, B_w1, B_w2, gw)
        return out.reshape(1, S, D)
    return f


_impl = make_kernel()


@jax.jit
def pallas_gated_mix__softmax_full_mha__dense_activation_relu__prompt_kernel(
    A_x: jax.Array,
    A_wqkv: jax.Array,
    A_wo: jax.Array,
    B_x: jax.Array,
    B_w1: jax.Array,
    B_w2: jax.Array,
    gate_w: jax.Array,
):
    return _impl(A_x, A_wqkv, A_wo, B_x, B_w1, B_w2, gate_w)
```

```python
import math
import jax
import jax.numpy as jnp
from jax import lax
import jax.experimental.pallas as pl
import jax.experimental.pallas.tpu as pltpu

S, D, H, DH, DFF = 2048, 640, 32, 20, 1536
HP = 24
HPS = 6
NSLAB = 6
SLABW = HPS * DH
F32 = jnp.float32
BF16 = jnp.bfloat16


def pk(x):
    return pltpu.bitcast(x, F32)


def upk(x):
    return pltpu.bitcast(x, BF16)


def zds(z, off, n):
    if isinstance(z, int):
        return pl.ds(z + off, n)
    return pl.ds(pl.multiple_of(z * 8 + off, 8), n)


NT = (((1,), (1,)), ((), ()))
TN = (((0,), (0,)), ((), ()))


def make_kernel(TQ=512, KC=128, PK=16, FORCE_FB=0, NP=4, NG=2, FB=256, WB=2):
    RB = TQ
    NB = S // RB
    NQ = S // TQ
    NFB = S // FB
    NSTEP = H * NQ
    NKC = S // KC
    NPER = -(-NKC // NP)
    HK = KC // 2
    KM = KC - PK
    C = (DH ** -0.5) * math.log2(math.e)
    U = 2 * NQ
    NIT = NSTEP // U
    FR = S // NIT
    QBR = (DH + 1) * 8

    def kernel(x_hbm, wqkv_hbm, wo_hbm, w1_hbm, w2_hbm, gw_ref, out_hbm,
               x_ref, wqkv_ref, wo_ref, w1_ref, w2_ref, out_ref,
               wqvt_ref, w1p_ref, w2p_ref, k_ref, qt_ref, vt_ref, ot_ref, bm_ref, g_ref,
               qz_ref, qb0_ref, qb1_ref, kb0_ref, kb1_ref, p0, p1, p2, p3,
               sem_in, sem_x, sem_out):
        kbbuf = (kb0_ref, kb1_ref)
        qbbuf = (qb0_ref, qb1_ref)
        pbuf = (p0, p1, p2, p3)

        def wq_cp(c0, c1, n):
            return pltpu.make_async_copy(wqkv_hbm.at[:, c0:c1], wqkv_ref.at[:, c0:c1], sem_in.at[n])
        cp_wk = wq_cp(D, 2 * D, 0)
        cp_wq = wq_cp(0, D, 1)
        cp_wv = wq_cp(2 * D, 3 * D, 2)
        cp_x = [pltpu.make_async_copy(x_hbm.at[i * RB:(i + 1) * RB], x_ref.at[i * RB:(i + 1) * RB], sem_x.at[i])
                for i in range(NB)]
        cp_w = [pltpu.make_async_copy(a, b, sem_in.at[3 + n])
                for n, (a, b) in enumerate(((w1_hbm, w1_ref), (w2_hbm, w2_ref), (wo_hbm, wo_ref)))]
        cp_wk.start()
        cp_x[0].start()
        for pb in pbuf:
            pb[NPER * HK:2 * NPER * HK, :] = jnp.zeros((NPER * HK, TQ), F32)
        for i in range(NQ):
            qt_ref[NSLAB - 1, i, 40:120] = jnp.zeros((80, TQ), F32)
        cp_wk.wait()
        cp_x[1].start()

        klane = lax.broadcasted_iota(jnp.int32, (RB // 2, 128), 1)
        ones_pk = pk(jnp.where(lax.broadcasted_iota(jnp.int32, (RB, 128), 1) < SLABW + HPS, 1.0, 0.0).astype(BF16))
        g48r = lax.broadcasted_iota(jnp.int32, (8 * NSLAB, D), 0)
        g48c = lax.broadcasted_iota(jnp.int32, (8 * NSLAB, D), 1)
        g48h = (g48r // 8) * HPS + (g48r % 8)
        g48 = jnp.where((g48c >= g48h * DH) & (g48c < g48h * DH + DH) & (g48r % 8 < HPS), 1.0, 0.0).astype(BF16)
        r8 = lax.broadcasted_iota(jnp.int32, (8, RB), 0)

        k2max = None
        for i in range(NB):
            if i == 0:
                cp_x[0].wait()
                cp_x[2].start()
                cp_x[3].start()
            if i == 1:
                cp_x[1].wait()
                cp_wq.start()
            if i == 2:
                cp_x[2].wait()
                cp_x[3].wait()
                cp_wq.wait()
                cp_wv.start()
                cp_w[0].start()
                cp_w[1].start()
            xb = x_ref[i * RB:(i + 1) * RB, :]
            ks = jnp.dot(xb, wqkv_ref[:, D:2 * D], preferred_element_type=F32)
            k2 = ks * ks
            k2max = k2 if k2max is None else jnp.maximum(k2max, k2)
            kp = pk(ks.astype(BF16))
            for j in range(NSLAB):
                sh = 8 * j
                if j == 0:
                    sl = kp[:, 0:128]
                elif j < NSLAB - 1:
                    sl = pltpu.roll(jnp.where(klane >= 128 - sh, kp[:, 128 * (j - 1):128 * j],
                                              kp[:, 128 * j:128 * (j + 1)]), sh, 1)
                else:
                    sl = pltpu.roll(jnp.where(klane >= 128 - sh, kp[:, 128 * (j - 1):128 * j], 0.0), sh, 1)
                k_ref[j, i * (RB // 2):(i + 1) * (RB // 2), :] = jnp.where(klane >= SLABW, ones_pk, sl)
            if i == 2:
                wqvt_ref[0:D, :] = wqkv_ref[:, 0:D].astype(F32).T.astype(BF16)
        kn = lax.dot_general(g48, k2max.astype(BF16), NT, preferred_element_type=F32)
        kmax = jnp.max(kn, axis=1, keepdims=True)

        def prep_jobs(h0, z):
            def tied(v, tie):
                if tie is None:
                    return v
                t = jnp.concatenate([tie] * (v.shape[1] // 128), axis=1)
                t = jnp.concatenate([t] * (v.shape[0] // 8), axis=0)
                return jnp.where(z == 0, v, t)
            jobs = []
            for par in range(2):
                h = h0 + par
                j = h // HPS
                i6 = h % HPS
                lo = i6 * DH
                for c in range(NKC):
                    qi = c // 4
                    part = c % 4

                    def kjob(tie, c=c, par=par, j=j, lo=lo):
                        kk = tied(k_ref[j, c * HK + KM // 2:(c + 1) * HK, :], tie)
                        k = pltpu.roll(upk(kk).astype(F32), (128 - lo) % 128, 1)
                        for d in range(DH):
                            kbbuf[par][zds(z, (d * NKC + c) * PK, PK), :] = jnp.broadcast_to(k[:, d:d + 1], (PK, 128))
                    jobs.append((40, "k", kjob))
                    for d in range(part * (DH + 1) // 4, (part + 1) * (DH + 1) // 4):
                        def qjob(tie, d=d, qi=qi, par=par, j=j, lo=lo, i6=i6):
                            r = lo + d if d < DH else SLABW + i6
                            v = jnp.broadcast_to(qt_ref[j, qi, pl.ds(r, 1), :], (8, TQ))
                            qbbuf[par][zds(z, qi * QBR + 8 * d, 8), :] = tied(v, tie)
                        jobs.append((4, "q", qjob))

                    def zjob(tie, part=part, qi=qi, par=par, j=j, lo=lo, i6=i6):
                        n = 32
                        q = qt_ref[j, qi, part * n:(part + 1) * n, :]
                        qr = lax.broadcasted_iota(jnp.int32, (n, TQ), 0) + part * n
                        keep = ((qr >= lo) & (qr < lo + DH)) | (qr == SLABW + i6)
                        v = pk(jnp.where(keep, q, 0.0).astype(BF16))
                        qz_ref[zds(z, (par * NQ + qi) * 64 + part * 16, 16), :] = tied(v, tie)
                    jobs.append((8, "q", zjob))
            return jobs

        jobs0 = prep_jobs(0, 0)
        kjobs0 = [f for _, kd, f in jobs0 if kd == "k"]
        qjobs0 = [f for _, kd, f in jobs0 if kd == "q"]

        for i in range(NB):
            xb = x_ref[i * RB:(i + 1) * RB, :]
            if i == WB:
                cp_wv.wait()
                cp_w[0].wait()
                cp_w[1].wait()
                cp_w[2].start()
                w1p_ref[...] = pk(w1_ref[...])
                w2p_ref[...] = pk(w2_ref[...])
                wqvt_ref[D:2 * D, :] = wqkv_ref[:, 2 * D:3 * D].astype(F32).T.astype(BF16)
            q = lax.dot_general(wqvt_ref[0:D, :], xb, NT, preferred_element_type=F32)
            q = (q * C).astype(BF16).astype(F32)
            qn = jnp.dot(g48, (q * q).astype(BF16), preferred_element_type=F32)
            nub = (-(jnp.sqrt(qn * kmax) * 1.03)).astype(BF16).astype(F32)
            for j in range(NSLAB):
                nv = min(SLABW, D - SLABW * j)
                qt_ref[j, i, 0:nv] = q[SLABW * j:SLABW * j + nv]
                qt_ref[j, i, SLABW:128] = nub[8 * j:8 * j + 8]
            for f_ in kjobs0[i * 8:(i + 1) * 8]:
                f_(None)

        gw16 = jnp.broadcast_to(gw_ref[...].astype(F32).reshape(1, D), (16, D)).astype(BF16)
        for i in range(NB):
            cs = slice(i * RB, (i + 1) * RB)
            xb = x_ref[cs, :]
            v = lax.dot_general(jnp.concatenate([wqvt_ref[D:, :], gw16], axis=0), xb, NT, preferred_element_type=F32)
            for p in range(H // 2):
                g = v[40 * p:40 * p + 40]
                mid = g[16:24]
                vt_ref[48 * p:48 * p + 16, cs] = g[0:16]
                vt_ref[48 * p + 16:48 * p + 24, cs] = jnp.where(r8 < 4, mid, jnp.where(r8 == 4, 1.0, 0.0))
                vt_ref[48 * p + 24:48 * p + 32, cs] = jnp.where(r8 >= 4, mid, jnp.where(r8 == 0, 1.0, 0.0))
                vt_ref[48 * p + 32:48 * p + 48, cs] = g[24:40]
            grow = jax.nn.sigmoid(v[D:D + 8])
            for t in range(RB // 128):
                gb = jnp.concatenate([grow[:, 128 * t:128 * (t + 1)]] * 16, axis=0)
                g_ref[i * RB + 128 * t:i * RB + 128 * (t + 1), :] = gb.T
            if i == 2:
                for f_ in qjobs0:
                    f_(None)

        qrow = lax.broadcasted_iota(jnp.int32, (128, TQ), 0)
        lastacc = [None]

        def stage(h, qi, cur, par, prev, z, z2, do_a=True):
            hp, qp, orow = prev
            vrow = pl.multiple_of(hp * HP, 8)
            acc = None
            wbase = (cur % 2) * NPER * HK
            rbase = ((cur + 1) % 2) * NPER * HK
            if do_a:
                ztrue = z2 == 0
                j = h // HPS
            for c in range(NKC):
                vt = vt_ref[pl.ds(vrow, HP), c * KC:(c + 1) * KC]
                pw = pbuf[c % NP][zds(z2, rbase + (c // NP) * HK, HK), :]
                d = jnp.dot(vt, upk(pw), preferred_element_type=F32)
                if acc is None:
                    acc = d if lastacc[0] is None else jnp.where(ztrue, d, lastacc[0])
                else:
                    acc = acc + d
                if not do_a:
                    continue
                s = jnp.dot(upk(k_ref[j, c * HK:c * HK + KM // 2, :]), upk(qz_ref[zds(z2, cur * 64, 64), :]),
                            preferred_element_type=F32)
                pbuf[c % NP][zds(z, wbase + (c // NP) * HK, KM // 2), :] = pk(jnp.exp2(s).astype(BF16))
                if PK:
                    GW = TQ // NG
                    tprev = None
                    for g in range(NG):
                        def ldq(dd):
                            v = qbbuf[par][zds(z2, qi * QBR + 8 * dd, 8), g * GW:(g + 1) * GW]
                            return jnp.concatenate([v] * (PK // 8), axis=0)
                        t = ldq(DH)
                        if tprev is not None:
                            t = jnp.where(ztrue, t, tprev)
                        for dd in range(DH):
                            kb = kbbuf[par][zds(z2, (dd * NKC + c) * PK, PK), :]
                            kb = jnp.concatenate([kb] * (GW // 128), axis=1)
                            t = t + kb * ldq(dd)
                        pbuf[c % NP][zds(z, wbase + (c // NP) * HK + KM // 2, PK // 2), g * GW:(g + 1) * GW] = pk(
                            jnp.exp2(t).astype(BF16))
                        tprev = t
            ot_ref[pl.ds(pl.multiple_of(orow, 8), HP), qp * TQ:(qp + 1) * TQ] = acc
            lastacc[0] = acc

        def body(u, c):
            z = lax.shift_right_logical(u, 8)
            z2 = lax.shift_right_logical(u, 9)
            lastacc[0] = None
            for i in range(U):
                h = 2 * u + i // NQ
                qi = i % NQ
                if i == 0:
                    hp = jnp.maximum(2 * u - 1, 0)
                    prev = (hp, NQ - 1, jnp.where(u == 0, H * HP, hp * HP))
                else:
                    hp = 2 * u + (i - 1) // NQ
                    prev = (hp, (i - 1) % NQ, hp * HP)
                stage(h, qi, i, (i // NQ) % 2, prev, z, z2)
            rs = pl.ds(pl.multiple_of(u * FR, FR), FR)
            xb = x_ref[rs, :]
            jobs = prep_jobs(jnp.minimum(2 * u + 2, H - 2), z)
            tot = sum(jb[0] for jb in jobs)
            durs = [640, 640, 384, 384, 384, 384, 288]
            cum = [sum(durs[:i + 1]) / sum(durs) for i in range(len(durs))]
            state = dict(i=0, acc=0)

            def release(k, val):
                nr = val.shape[0] // 8
                nv = nr * (val.shape[1] // 128)
                while state["i"] < len(jobs) and (state["acc"] + jobs[state["i"]][0] / 2) / tot <= cum[k]:
                    cst, _, fn = jobs[state["i"]]
                    lo_ = cum[k - 1] if k else 0.0
                    frac = min(max((state["acc"] / tot - lo_) / (cum[k] - lo_), 0.0), 0.999)
                    col, row = divmod(int(frac * nv), nr)
                    fn(val[8 * row:8 * row + 8, 128 * col:128 * (col + 1)])
                    state["i"] += 1
                    state["acc"] += cst
            hs = []
            for n in range(3):
                w = w1p_ref[:, 512 * n:512 * (n + 1)]
                rows = [w[64 * t:64 * (t + 1)] for t in range(5)]
                for (t, a_) in {0: [(4, 0)], 1: [(0, 1), (2, 2), (4, 3)]}.get(n, []):
                    top = jnp.where(z2 == 0, rows[t][0:8], pbuf[a_][zds(z2, 0, 8), :])
                    rows[t] = jnp.concatenate([top, rows[t][8:]], axis=0)
                w = jnp.concatenate(rows, axis=0)
                hf = jnp.maximum(jnp.dot(xb, upk(w), preferred_element_type=F32), 0.0)
                release(n, hf)
                hs.append(hf.astype(BF16))
            h1 = jnp.concatenate(hs, axis=1)
            g1 = 1.0 - g_ref[rs, :]
            for n in range(5):
                bn = jnp.dot(h1, upk(w2p_ref[:, 128 * n:128 * (n + 1)]), preferred_element_type=F32)
                if n < 4:
                    release(3 + n, bn)
                bm_ref[rs, 128 * n:128 * (n + 1)] = g1 * bn
            assert state["i"] == len(jobs)
            return c
        lax.fori_loop(0, NIT, body, 0)
        lastacc[0] = None
        stage(0, 0, 0, 0, (H - 1, NQ - 1, (H - 1) * HP), 0, 0, do_a=False)

        cp_w[2].wait()

        def out_cp(i):
            rs = pl.ds(i * FB, FB) if isinstance(i, int) else pl.ds(pl.multiple_of(i * FB, FB), FB)
            return pltpu.make_async_copy(out_ref.at[rs], out_hbm.at[rs], sem_out.at[i])

        r8f = lax.broadcasted_iota(jnp.int32, (8, FB), 0)

        def fin(i, check):
            rs = pl.ds(i * FB, FB) if isinstance(i, int) else pl.ds(pl.multiple_of(i * FB, FB), FB)
            parts = []
            lmin = lmax = None
            for p in range(H // 2):
                e = ot_ref[48 * p:48 * p + 24, rs]
                o = ot_ref[48 * p + 24:48 * p + 48, rs]
                if check:
                    l = jnp.where(r8f < 4, o[0:8], e[16:24])
                    lmin = l if lmin is None else jnp.minimum(lmin, l)
                    lmax = l if lmax is None else jnp.maximum(lmax, l)
                e = e * (1.0 / e[DH:DH + 1])
                o = o * (1.0 / o[0:1])
                parts += [e[0:16], jnp.where(r8f < 4, e[16:24], o[0:8]), o[8:24]]
            ot = jnp.concatenate(parts, axis=0).astype(BF16)
            a = lax.dot_general(ot, wo_ref[...], TN, preferred_element_type=F32)
            g = jnp.concatenate([g_ref[rs, :]] * (D // 128), axis=1)
            out_ref[rs, :] = (g * a + bm_ref[rs, :]).astype(out_ref.dtype)
            out_cp(i).start()
            if check:
                ok = (lmin >= 2.0 ** -60) & (lmax <= 4096.0)
                return jnp.where(ok | ((r8f != 0) & (r8f != 4)), 0.0, 1.0)

        bad = None
        for i in range(NFB):
            bi = fin(i, True)
            bad = bi if bad is None else jnp.maximum(bad, bi)
        nbad = jnp.max(jnp.max(bad, axis=1, keepdims=True), axis=0, keepdims=True)[0, 0]
        if FORCE_FB:
            nbad = nbad + 1.0
        for i in range(NFB):
            out_cp(i).wait()

        @pl.when(nbad > 0.0)
        def _():
            def fb(t, c):
                h = t // NQ
                qi = t % NQ
                j = h // HPS
                lo = (h % HPS) * DH
                qz = jnp.where((qrow >= lo) & (qrow < lo + DH), qt_ref[j, qi], 0.0).astype(BF16)
                s = jnp.dot(upk(k_ref[j]), qz, preferred_element_type=F32)
                m = jnp.max(s, axis=0, keepdims=True)
                p = jnp.exp2(s - m).astype(BF16)
                vrow = pl.multiple_of(h * HP, 8)
                acc = jnp.dot(vt_ref[pl.ds(vrow, HP), :], p, preferred_element_type=F32)
                ot_ref[pl.ds(vrow, HP), pl.ds(pl.multiple_of(qi * TQ, TQ), TQ)] = acc
                return c
            lax.fori_loop(0, NSTEP, fb, 0)

            def fin2(i, c):
                fin(i, False)
                out_cp(i).wait()
                return c
            lax.fori_loop(0, NFB, fin2, 0)

    PKP = max(PK, 8)
    scratch = [
        pltpu.VMEM((S, D), BF16),
        pltpu.VMEM((D, 3 * D), BF16),
        pltpu.VMEM((D, D), BF16),
        pltpu.VMEM((D, DFF), BF16),
        pltpu.VMEM((DFF, D), BF16),
        pltpu.VMEM((S, D), BF16),
        pltpu.VMEM((2 * D, D), BF16),
        pltpu.VMEM((D // 2, DFF), F32),
        pltpu.VMEM((DFF // 2, D), F32),
        pltpu.VMEM((NSLAB, S // 2, 128), F32),
        pltpu.VMEM((NSLAB, NQ, 128, TQ), F32),
        pltpu.VMEM((H * HP, S), F32),
        pltpu.VMEM((H * HP + HP, S), F32),
        pltpu.VMEM((S, D), F32),
        pltpu.VMEM((S, 128), F32),
        pltpu.VMEM((U * 64, TQ), F32),
        pltpu.VMEM((NQ * QBR, TQ), F32),
        pltpu.VMEM((NQ * QBR, TQ), F32),
        pltpu.VMEM((DH * NKC * PKP, 128), F32),
        pltpu.VMEM((DH * NKC * PKP, 128), F32),
    ] + [pltpu.VMEM((2 * NPER * HK, TQ), F32)] * NP + [
        pltpu.SemaphoreType.DMA((6,)),
        pltpu.SemaphoreType.DMA((NB,)),
        pltpu.SemaphoreType.DMA((NFB,)),
    ]
    anyspec = pl.BlockSpec(memory_space=pl.ANY)

    @jax.jit
    def f(A_x, A_wqkv, A_wo, B_x, B_w1, B_w2, gate_w):
        x = A_x.reshape(S, D)
        out = pl.pallas_call(
            kernel,
            out_shape=jax.ShapeDtypeStruct((S, D), BF16),
            in_specs=[anyspec] * 5 + [pl.BlockSpec(memory_space=pltpu.VMEM)],
            out_specs=anyspec,
            scratch_shapes=scratch,
            compiler_params=pltpu.CompilerParams(vmem_limit_bytes=100 * 1024 * 1024),
        )(x, A_wqkv, A_wo, B_w1, B_w2, gate_w)
        return out.reshape(1, S, D)
    return f


_impl = make_kernel()


@jax.jit
def pallas_gated_mix__softmax_full_mha__dense_activation_relu__prompt_kernel(
    A_x: jax.Array,
    A_wqkv: jax.Array,
    A_wo: jax.Array,
    B_x: jax.Array,
    B_w1: jax.Array,
    B_w2: jax.Array,
    gate_w: jax.Array,
):
    return _impl(A_x, A_wqkv, A_wo, B_x, B_w1, B_w2, gate_w)
```

```python
import math

import jax
import jax.numpy as jnp
from jax import lax
import jax.experimental.pallas as pl
import jax.experimental.pallas.tpu as pltpu

S, D, H, DH, DFF = 2048, 640, 32, 20, 1536
HP = 24
HPS = 6
NSLAB = 6
SLABW = HPS * DH
F32 = jnp.float32
BF16 = jnp.bfloat16

TQ = 512
KC = 128
PK = 16
NP = 4
NG = 2
FB = 128
RB = TQ
NB = S // RB
NQ = S // TQ
NFB = S // FB
NSTEP = H * NQ
NKC = S // KC
NPER = NKC // NP
HK = KC // 2
KM = KC - PK
U = 2 * NQ
NIT = NSTEP // U
FR = S // NIT
QBR = (DH + 1) * 8
GW = TQ // NG
QSCALE = (DH ** -0.5) * math.log2(math.e)

NT = (((1,), (1,)), ((), ()))
TN = (((0,), (0,)), ((), ()))


def pk(x):
    return pltpu.bitcast(x, F32)


def upk(x):
    return pltpu.bitcast(x, BF16)


def zds(z, off, n):
    if isinstance(z, int):
        return pl.ds(z + off, n)
    return pl.ds(pl.multiple_of(z * 8 + off, 8), n)


def tied(v, tie, zt):
    if tie is None:
        return v
    t = jnp.concatenate([tie] * (v.shape[1] // 128), axis=1)
    t = jnp.concatenate([t] * (v.shape[0] // 8), axis=0)
    if zt.ndim:
        m = jnp.concatenate([zt] * (v.shape[1] // 128), axis=1)
        m = jnp.concatenate([m] * (v.shape[0] // 8), axis=0)
        return jnp.where(m != 0, v, t)
    return jnp.where(zt == 0, v, t)


def spread(fns, val):
    nr = val.shape[0] // 8
    nv = nr * (val.shape[1] // 128)
    for n_, fn in enumerate(fns):
        col, row = divmod((n_ * nv) // len(fns), nr)
        fn(val[8 * row:8 * row + 8, 128 * col:128 * (col + 1)])


def _kernel(x_hbm, wqkv_hbm, wo_hbm, w1_hbm, w2_hbm, gw_ref, out_hbm,
            x_ref, wq_ref, wk_ref, wv_ref, wo_ref, w1_ref, w2_ref, out_ref,
            wqvt_ref, w1p_ref, w2p_ref, k_ref, qt_ref, vt_ref, ot_ref, bm_ref, g_ref,
            qz_ref, qb0_ref, qb1_ref, kb0_ref, kb1_ref, p0, p1, p2, p3,
            sem_in, sem_x, sem_out):
    kbbuf = (kb0_ref, kb1_ref)
    qbbuf = (qb0_ref, qb1_ref)
    pbuf = (p0, p1, p2, p3)

    cp_wk = pltpu.make_async_copy(wqkv_hbm.at[:, D:2 * D], wk_ref, sem_in.at[0])
    cp_wq = pltpu.make_async_copy(wqkv_hbm.at[:, 0:D], wq_ref, sem_in.at[1])
    cp_wv = pltpu.make_async_copy(wqkv_hbm.at[:, 2 * D:3 * D], wv_ref, sem_in.at[2])
    cp_x = [pltpu.make_async_copy(x_hbm.at[i * RB:(i + 1) * RB], x_ref.at[i * RB:(i + 1) * RB], sem_x.at[i])
            for i in range(NB)]
    cp_w = [pltpu.make_async_copy(a, b, sem_in.at[3 + n])
            for n, (a, b) in enumerate(((w1_hbm, w1_ref), (w2_hbm, w2_ref), (wo_hbm, wo_ref)))]
    cp_wk.start()
    cp_x[0].start()
    for pb in pbuf:
        pb[NPER * HK:2 * NPER * HK, :] = jnp.zeros((NPER * HK, TQ), F32)
    for i in range(NQ):
        qt_ref[NSLAB - 1, i, 40:120] = jnp.zeros((80, TQ), F32)
    cp_wk.wait()
    cp_x[1].start()

    klane = lax.broadcasted_iota(jnp.int32, (RB // 2, 128), 1)
    ones_pk = pk(jnp.where(lax.broadcasted_iota(jnp.int32, (RB, 128), 1) < SLABW + HPS, 1.0, 0.0).astype(BF16))
    g48r = lax.broadcasted_iota(jnp.int32, (8 * NSLAB, D), 0)
    g48c = lax.broadcasted_iota(jnp.int32, (8 * NSLAB, D), 1)
    g48h = (g48r // 8) * HPS + (g48r % 8)
    g48 = jnp.where((g48c >= g48h * DH) & (g48c < g48h * DH + DH) & (g48r % 8 < HPS), 1.0, 0.0).astype(BF16)
    r8 = lax.broadcasted_iota(jnp.int32, (8, RB), 0)

    kamax = None
    for i in range(NB):
        if i == 0:
            cp_x[0].wait()
            cp_x[2].start()
            cp_x[3].start()
        if i == 1:
            cp_x[1].wait()
            cp_wq.start()
        if i == 2:
            cp_x[2].wait()
            cp_x[3].wait()
            cp_wq.wait()
            cp_wv.start()
            cp_w[0].start()
            cp_w[1].start()
        xb = x_ref[i * RB:(i + 1) * RB, :]
        ks = jnp.concatenate(
            [jnp.dot(xb[t * 128:(t + 1) * 128], wk_ref[...], preferred_element_type=F32)
             for t in range(RB // 128)], axis=0)
        ka = jnp.max(jnp.abs(ks).reshape(RB // 8, 8, D), axis=0)
        kamax = ka if kamax is None else jnp.maximum(kamax, ka)
        kp = pk(ks.astype(BF16))
        for j in range(NSLAB):
            sh = 8 * j
            if j == 0:
                sl = kp[:, 0:128]
            elif j < NSLAB - 1:
                sl = pltpu.roll(jnp.where(klane >= 128 - sh, kp[:, 128 * (j - 1):128 * j],
                                          kp[:, 128 * j:128 * (j + 1)]), sh, 1)
            else:
                sl = pltpu.roll(jnp.where(klane >= 128 - sh, kp[:, 128 * (j - 1):128 * j], 0.0), sh, 1)
            k_ref[j, i * (RB // 2):(i + 1) * (RB // 2), :] = jnp.where(klane >= SLABW, ones_pk, sl)
        if i == 2:
            wqvt_ref[0:D, :] = wq_ref[...].astype(F32).T.astype(BF16)
    k2 = jnp.concatenate([kamax * kamax] * 16, axis=0)
    kn = lax.dot_general(g48, k2.astype(BF16), NT, preferred_element_type=F32)
    kmax = jnp.max(kn, axis=1, keepdims=True)

    def prep_jobs(h0, z, zt):
        jobs = []
        for par in range(2):
            h = h0 + par
            j = h // HPS
            i6 = h % HPS
            lo = i6 * DH
            for c in range(NKC):
                qi = c // 4
                part = c % 4

                def kjob(tie, c=c, par=par, j=j, lo=lo):
                    kk = tied(k_ref[j, c * HK + KM // 2:(c + 1) * HK, :], tie, zt)
                    k = pltpu.roll(upk(kk).astype(F32), (128 - lo) % 128, 1)
                    for d in range(DH):
                        kbbuf[par][zds(z, (d * NKC + c) * PK, PK), :] = jnp.broadcast_to(k[:, d:d + 1], (PK, 128))
                jobs.append((40, "k", kjob))
                for d in range(part * (DH + 1) // 4, (part + 1) * (DH + 1) // 4):
                    def qjob(tie, d=d, qi=qi, par=par, j=j, lo=lo, i6=i6):
                        r = lo + d if d < DH else SLABW + i6
                        v = jnp.broadcast_to(qt_ref[j, qi, pl.ds(r, 1), :], (8, TQ))
                        qbbuf[par][zds(z, qi * QBR + 8 * d, 8), :] = tied(v, tie, zt)
                    jobs.append((4, "q", qjob))

                def zjob(tie, part=part, qi=qi, par=par, j=j, lo=lo, i6=i6):
                    n = 32
                    q = qt_ref[j, qi, part * n:(part + 1) * n, :]
                    qr = lax.broadcasted_iota(jnp.int32, (n, TQ), 0) + part * n
                    keep = ((qr >= lo) & (qr < lo + DH)) | (qr == SLABW + i6)
                    v = pk(jnp.where(keep, q, 0.0).astype(BF16))
                    qz_ref[zds(z, (par * NQ + qi) * 64 + part * 16, 16), :] = tied(v, tie, zt)
                jobs.append((8, "q", zjob))
        return jobs

    z0 = lax.bitcast_convert_type(k_ref[0, 0:8, :], jnp.int32) | 1
    jobs0 = prep_jobs(0, 0, z0)
    kjobs0 = [f for _, kd, f in jobs0 if kd == "k"]
    qjobs0 = [f for _, kd, f in jobs0 if kd == "q"]
    wjobs = []
    for r in range(D // 16):
        def w1job(tie, r=r):
            w1p_ref[8 * r:8 * r + 8, :] = tied(pk(w1_ref[16 * r:16 * r + 16, :]), tie, z0)
        wjobs.append(w1job)
    for r in range(DFF // 32):
        def w2job(tie, r=r):
            w2p_ref[16 * r:16 * r + 16, :] = tied(pk(w2_ref[32 * r:32 * r + 32, :]), tie, z0)
        wjobs.append(w2job)

    for i in range(NB):
        xb = x_ref[i * RB:(i + 1) * RB, :]
        if i == 2:
            cp_wv.wait()
            cp_w[0].wait()
            cp_w[1].wait()
            cp_w[2].start()
            wqvt_ref[D:2 * D, :] = wv_ref[...].astype(F32).T.astype(BF16)
        q = lax.dot_general(wqvt_ref[0:D, :], xb, NT, preferred_element_type=F32)
        q = (q * QSCALE).astype(BF16).astype(F32)
        qn = jnp.dot(g48, (q * q).astype(BF16), preferred_element_type=F32)
        nshift = (jnp.sqrt(qn * kmax) * -0.25).astype(BF16).astype(F32)
        for j in range(NSLAB):
            nv = min(SLABW, D - SLABW * j)
            qt_ref[j, i, 0:nv] = q[SLABW * j:SLABW * j + nv]
            qt_ref[j, i, SLABW:128] = nshift[8 * j:8 * j + 8]
        for f_ in kjobs0[i * 8:(i + 1) * 8]:
            f_(None)
        if i >= 2:
            spread(wjobs[(i - 2) * 44:(i - 1) * 44], q)

    gw16 = jnp.broadcast_to(gw_ref[...].astype(F32).reshape(1, D), (16, D)).astype(BF16)
    for i in range(NB):
        cs = slice(i * RB, (i + 1) * RB)
        xb = x_ref[cs, :]
        v = lax.dot_general(jnp.concatenate([wqvt_ref[D:, :], gw16], axis=0), xb, NT, preferred_element_type=F32)
        for p in range(H // 2):
            g = v[40 * p:40 * p + 40]
            mid = g[16:24]
            vt_ref[48 * p:48 * p + 16, cs] = g[0:16]
            vt_ref[48 * p + 16:48 * p + 24, cs] = jnp.where(r8 < 4, mid, jnp.where(r8 == 4, 1.0, 0.0))
            vt_ref[48 * p + 24:48 * p + 32, cs] = jnp.where(r8 >= 4, mid, jnp.where(r8 == 0, 1.0, 0.0))
            vt_ref[48 * p + 32:48 * p + 48, cs] = g[24:40]
        grow = jax.nn.sigmoid(v[D:D + 8])
        for t in range(RB // 128):
            gb = jnp.concatenate([grow[:, 128 * t:128 * (t + 1)]] * 16, axis=0)
            g_ref[i * RB + 128 * t:i * RB + 128 * (t + 1), :] = gb.T
        if i < 3:
            spread(qjobs0[i * len(qjobs0) // 3:(i + 1) * len(qjobs0) // 3], v[0:D])

    lastacc = [None]

    def stage(h, qi, cur, par, prev, z, z2, do_a=True):
        hp, qp, orow = prev
        vrow = pl.multiple_of(hp * HP, 8)
        acc = None
        wbase = (cur % 2) * NPER * HK
        rbase = ((cur + 1) % 2) * NPER * HK
        if do_a:
            ztrue = z2 == 0
            j = h // HPS
        for c in range(NKC):
            vt = vt_ref[pl.ds(vrow, HP), c * KC:(c + 1) * KC]
            pw = pbuf[c % NP][zds(z2, rbase + (c // NP) * HK, HK), :]
            d = jnp.dot(vt, upk(pw), preferred_element_type=F32)
            if acc is None:
                acc = d if lastacc[0] is None else jnp.where(ztrue, d, lastacc[0])
            else:
                acc = acc + d
            if not do_a:
                continue
            s = jnp.dot(upk(k_ref[j, c * HK:c * HK + KM // 2, :]), upk(qz_ref[zds(z2, cur * 64, 64), :]),
                        preferred_element_type=F32)
            pbuf[c % NP][zds(z, wbase + (c // NP) * HK, KM // 2), :] = pk(jnp.exp2(s).astype(BF16))
            tprev = None
            for g in range(NG):
                def ldq(dd):
                    v = qbbuf[par][zds(z2, qi * QBR + 8 * dd, 8), g * GW:(g + 1) * GW]
                    return jnp.concatenate([v] * (PK // 8), axis=0)
                t = ldq(DH)
                if tprev is not None:
                    t = jnp.where(ztrue, t, tprev)
                for dd in range(DH):
                    kb = kbbuf[par][zds(z2, (dd * NKC + c) * PK, PK), :]
                    kb = jnp.concatenate([kb] * (GW // 128), axis=1)
                    t = t + kb * ldq(dd)
                pbuf[c % NP][zds(z, wbase + (c // NP) * HK + KM // 2, PK // 2), g * GW:(g + 1) * GW] = pk(
                    jnp.exp2(t).astype(BF16))
                tprev = t
        ot_ref[pl.ds(pl.multiple_of(orow, 8), HP), qp * TQ:(qp + 1) * TQ] = acc
        lastacc[0] = acc

    def body(u, carry):
        z = lax.shift_right_logical(u, 8)
        z2 = lax.shift_right_logical(u, 9)
        lastacc[0] = None
        for i in range(U):
            h = 2 * u + i // NQ
            qi = i % NQ
            if i == 0:
                hp = jnp.maximum(2 * u - 1, 0)
                prev = (hp, NQ - 1, jnp.where(u == 0, H * HP, hp * HP))
            else:
                hp = 2 * u + (i - 1) // NQ
                prev = (hp, (i - 1) % NQ, hp * HP)
            stage(h, qi, i, (i // NQ) % 2, prev, z, z2)

        rs = pl.ds(pl.multiple_of(u * FR, FR), FR)
        xb = x_ref[rs, :]
        jobs = prep_jobs(jnp.minimum(2 * u + 2, H - 2), z, z)
        tot = sum(jb[0] for jb in jobs)
        durs = [640, 640] + [128] * 14
        cum = [sum(durs[:i + 1]) / sum(durs) for i in range(len(durs))]
        state = dict(i=0, acc=0)

        def release(k, val):
            nr = val.shape[0] // 8
            nv = nr * (val.shape[1] // 128)
            while state["i"] < len(jobs) and (state["acc"] + jobs[state["i"]][0] / 2) / tot <= cum[k]:
                cst, _, fn = jobs[state["i"]]
                lo_ = cum[k - 1] if k else 0.0
                frac = min(max((state["acc"] / tot - lo_) / (cum[k] - lo_), 0.0), 0.999)
                col, row = divmod(int(frac * nv), nr)
                fn(val[8 * row:8 * row + 8, 128 * col:128 * (col + 1)])
                state["i"] += 1
                state["acc"] += cst
        hs = []
        for n in range(3):
            w = w1p_ref[:, 512 * n:512 * (n + 1)]
            rows = [w[64 * t:64 * (t + 1)] for t in range(5)]
            for (t, a_) in {0: [(4, 0)], 1: [(0, 1), (2, 2), (4, 3)]}.get(n, []):
                top = jnp.where(z2 == 0, rows[t][0:8], pbuf[a_][zds(z2, 0, 8), :])
                rows[t] = jnp.concatenate([top, rows[t][8:]], axis=0)
            w = jnp.concatenate(rows, axis=0)
            hf = jnp.maximum(jnp.dot(xb, upk(w), preferred_element_type=F32), 0.0)
            release(n, hf)
            hs.append(hf.astype(BF16))
        g1 = 1.0 - g_ref[rs, :]
        for n in range(5):
            bn = None
            for kk in range(3):
                pd = jnp.dot(hs[kk], upk(w2p_ref[256 * kk:256 * (kk + 1), 128 * n:128 * (n + 1)]),
                             preferred_element_type=F32)
                bn = pd if bn is None else bn + pd
                if 3 + n * 3 + kk < len(durs):
                    release(3 + n * 3 + kk, pd)
            bm_ref[rs, 128 * n:128 * (n + 1)] = g1 * bn
        assert state["i"] == len(jobs)
        return carry
    lax.fori_loop(0, NIT, body, 0)
    lastacc[0] = None
    stage(0, 0, 0, 0, (H - 1, NQ - 1, (H - 1) * HP), 0, 0, do_a=False)

    cp_w[2].wait()

    def rows_of(i):
        return pl.ds(i * FB, FB) if isinstance(i, int) else pl.ds(pl.multiple_of(i * FB, FB), FB)

    def out_cp(i):
        return pltpu.make_async_copy(out_ref.at[rows_of(i)], out_hbm.at[rows_of(i)], sem_out.at[i])

    r8f = lax.broadcasted_iota(jnp.int32, (8, FB), 0)

    def fin(i, check):
        rs = rows_of(i)
        parts = []
        lmin = amax = None
        for p in range(H // 2):
            e = ot_ref[48 * p:48 * p + 24, rs]
            o = ot_ref[48 * p + 24:48 * p + 48, rs]
            if check:
                l = jnp.where(r8f < 4, o[0:8], e[16:24])
                lmin = l if lmin is None else jnp.minimum(lmin, l)
                for t_ in (e, o):
                    am = jnp.max(jnp.abs(t_).reshape(3, 8, FB), axis=0)
                    amax = am if amax is None else jnp.maximum(amax, am)
            e = e * (1.0 / e[DH:DH + 1])
            o = o * (1.0 / o[0:1])
            parts += [e[0:16], jnp.where(r8f < 4, e[16:24], o[0:8]), o[8:24]]
        ot = jnp.concatenate(parts, axis=0).astype(BF16)
        a = lax.dot_general(ot, wo_ref[...], TN, preferred_element_type=F32)
        g = jnp.concatenate([g_ref[rs, :]] * (D // 128), axis=1)
        out_ref[rs, :] = (g * a + bm_ref[rs, :]).astype(out_ref.dtype)
        out_cp(i).start()
        if check:
            ok = ((lmin >= 2.0 ** -60) | ((r8f != 0) & (r8f != 4))) & (amax <= 2.0 ** 120)
            return jnp.where(ok, 0.0, 1.0)

    bad = None
    for i in range(NFB):
        bi = fin(i, True)
        bad = bi if bad is None else jnp.maximum(bad, bi)
    nbad = jnp.max(jnp.max(bad, axis=1, keepdims=True), axis=0, keepdims=True)[0, 0]
    for i in range(NFB):
        out_cp(i).wait()

    @pl.when(nbad > FORCE)
    def _():
        qrow = lax.broadcasted_iota(jnp.int32, (128, TQ), 0)

        def fb(t, c):
            h = t // NQ
            qi = t % NQ
            j = h // HPS
            lo = (h % HPS) * DH
            qz = jnp.where((qrow >= lo) & (qrow < lo + DH), qt_ref[j, qi], 0.0).astype(BF16)
            s = jnp.dot(upk(k_ref[j]), qz, preferred_element_type=F32)
            m = jnp.max(s, axis=0, keepdims=True)
            p = jnp.exp2(s - m).astype(BF16)
            vrow = pl.multiple_of(h * HP, 8)
            acc = jnp.dot(vt_ref[pl.ds(vrow, HP), :], p, preferred_element_type=F32)
            ot_ref[pl.ds(vrow, HP), pl.ds(pl.multiple_of(qi * TQ, TQ), TQ)] = acc
            return c
        lax.fori_loop(0, NSTEP, fb, 0)

        def fin2(i, c):
            fin(i, False)
            out_cp(i).wait()
            return c
        lax.fori_loop(0, NFB, fin2, 0)


FORCE = 0.0

_SCRATCH = [
    pltpu.VMEM((S, D), BF16),
    pltpu.VMEM((D, D), BF16),
    pltpu.VMEM((D, D), BF16),
    pltpu.VMEM((D, D), BF16),
    pltpu.VMEM((D, D), BF16),
    pltpu.VMEM((D, DFF), BF16),
    pltpu.VMEM((DFF, D), BF16),
    pltpu.VMEM((S, D), BF16),
    pltpu.VMEM((2 * D, D), BF16),
    pltpu.VMEM((D // 2, DFF), F32),
    pltpu.VMEM((DFF // 2, D), F32),
    pltpu.VMEM((NSLAB, S // 2, 128), F32),
    pltpu.VMEM((NSLAB, NQ, 128, TQ), F32),
    pltpu.VMEM((H * HP, S), F32),
    pltpu.VMEM((H * HP + HP, S), F32),
    pltpu.VMEM((S, D), F32),
    pltpu.VMEM((S, 128), F32),
    pltpu.VMEM((U * 64, TQ), F32),
    pltpu.VMEM((NQ * QBR, TQ), F32),
    pltpu.VMEM((NQ * QBR, TQ), F32),
    pltpu.VMEM((DH * NKC * PK, 128), F32),
    pltpu.VMEM((DH * NKC * PK, 128), F32),
] + [pltpu.VMEM((2 * NPER * HK, TQ), F32)] * NP + [
    pltpu.SemaphoreType.DMA((6,)),
    pltpu.SemaphoreType.DMA((NB,)),
    pltpu.SemaphoreType.DMA((NFB,)),
]


@jax.jit
def pallas_gated_mix__softmax_full_mha__dense_activation_relu__prompt_kernel(
    A_x: jax.Array,
    A_wqkv: jax.Array,
    A_wo: jax.Array,
    B_x: jax.Array,
    B_w1: jax.Array,
    B_w2: jax.Array,
    gate_w: jax.Array,
):
    anyspec = pl.BlockSpec(memory_space=pl.ANY)
    out = pl.pallas_call(
        _kernel,
        out_shape=jax.ShapeDtypeStruct((S, D), BF16),
        in_specs=[anyspec] * 5 + [pl.BlockSpec(memory_space=pltpu.VMEM)],
        out_specs=anyspec,
        scratch_shapes=_SCRATCH,
        compiler_params=pltpu.CompilerParams(vmem_limit_bytes=100 * 1024 * 1024),
    )(A_x.reshape(S, D), A_wqkv, A_wo, B_w1, B_w2, gate_w)
    return out.reshape(1, S, D)
```

```python
import math

import jax
import jax.numpy as jnp
from jax import lax
import jax.experimental.pallas as pl
import jax.experimental.pallas.tpu as pltpu

S, D, H, DH, DFF = 2048, 640, 32, 20, 1536
HP = 24
HPS = 6
NSLAB = 6
SLABW = HPS * DH
F32 = jnp.float32
BF16 = jnp.bfloat16

TQ = 512
KC = 128
PK = 16
NP = 4
NG = 2
FB = 128
RB = TQ
NB = S // RB
NQ = S // TQ
NFB = S // FB
NSTEP = H * NQ
NKC = S // KC
NPER = NKC // NP
HK = KC // 2
KM = KC - PK
U = 2 * NQ
NIT = NSTEP // U
FR = S // NIT
QBR = (DH + 1) * 8
GW = TQ // NG
QSCALE = (DH ** -0.5) * math.log2(math.e)

NT = (((1,), (1,)), ((), ()))
TN = (((0,), (0,)), ((), ()))


def pk(x):
    return pltpu.bitcast(x, F32)


def upk(x):
    return pltpu.bitcast(x, BF16)


def zview(ref, z):
    if isinstance(z, int):
        return ref
    return ref.at[pl.ds(pl.multiple_of(z * 8, 8), ref.shape[0])]


def tied(v, tie, zt):
    if tie is None:
        return v
    t = jnp.concatenate([tie] * (v.shape[1] // 128), axis=1)
    t = jnp.concatenate([t] * (v.shape[0] // 8), axis=0)
    if zt.ndim:
        m = jnp.concatenate([zt] * (v.shape[1] // 128), axis=1)
        m = jnp.concatenate([m] * (v.shape[0] // 8), axis=0)
        return jnp.where(m != 0, v, t)
    return jnp.where(zt == 0, v, t)


def spread(fns, val):
    nr = val.shape[0] // 8
    nv = nr * (val.shape[1] // 128)
    for n_, fn in enumerate(fns):
        col, row = divmod((n_ * nv) // len(fns), nr)
        fn(val[8 * row:8 * row + 8, 128 * col:128 * (col + 1)])


def _kernel(x_hbm, wqkv_hbm, wo_hbm, w1_hbm, w2_hbm, gw_ref, out_hbm,
            x_ref, wq_ref, wk_ref, wv_ref, wo_ref, w1_ref, w2_ref, out_ref,
            wqvt_ref, w1p_ref, w2p_ref, k_ref, qt_ref, vt_ref, ot_ref, bm_ref, g_ref,
            qz_ref, qb0_ref, qb1_ref, kb0_ref, kb1_ref, p0, p1, p2, p3,
            sem_in, sem_x, sem_out):
    kbbuf = (kb0_ref, kb1_ref)
    qbbuf = (qb0_ref, qb1_ref)
    pbuf = (p0, p1, p2, p3)

    cp_wk = pltpu.make_async_copy(wqkv_hbm.at[:, D:2 * D], wk_ref, sem_in.at[0])
    cp_wq = pltpu.make_async_copy(wqkv_hbm.at[:, 0:D], wq_ref, sem_in.at[1])
    cp_wv = pltpu.make_async_copy(wqkv_hbm.at[:, 2 * D:3 * D], wv_ref, sem_in.at[2])
    cp_x = [pltpu.make_async_copy(x_hbm.at[i * RB:(i + 1) * RB], x_ref.at[i * RB:(i + 1) * RB], sem_x.at[i])
            for i in range(NB)]
    cp_w = [pltpu.make_async_copy(a, b, sem_in.at[3 + n])
            for n, (a, b) in enumerate(((w1_hbm, w1_ref), (w2_hbm, w2_ref), (wo_hbm, wo_ref)))]
    cp_wk.start()
    cp_x[0].start()
    for pb in pbuf:
        pb[NPER * HK:2 * NPER * HK, :] = jnp.zeros((NPER * HK, TQ), F32)
    for i in range(NQ):
        qt_ref[NSLAB - 1, i, 40:120] = jnp.zeros((80, TQ), F32)
    cp_wk.wait()
    cp_x[1].start()

    klane = lax.broadcasted_iota(jnp.int32, (RB // 2, 128), 1)
    ones_pk = pk(jnp.where(lax.broadcasted_iota(jnp.int32, (RB, 128), 1) < SLABW + HPS, 1.0, 0.0).astype(BF16))
    g48r = lax.broadcasted_iota(jnp.int32, (8 * NSLAB, D), 0)
    g48c = lax.broadcasted_iota(jnp.int32, (8 * NSLAB, D), 1)
    g48h = (g48r // 8) * HPS + (g48r % 8)
    g48 = jnp.where((g48c >= g48h * DH) & (g48c < g48h * DH + DH) & (g48r % 8 < HPS), 1.0, 0.0).astype(BF16)
    r8 = lax.broadcasted_iota(jnp.int32, (8, RB), 0)

    kamax = None
    for i in range(NB):
        if i == 0:
            cp_x[0].wait()
            cp_x[2].start()
            cp_x[3].start()
        if i == 1:
            cp_x[1].wait()
            cp_wq.start()
        if i == 2:
            cp_x[2].wait()
            cp_x[3].wait()
            cp_wq.wait()
            cp_wv.start()
            cp_w[0].start()
            cp_w[1].start()
        xb = x_ref[i * RB:(i + 1) * RB, :]
        ks = jnp.concatenate(
            [jnp.dot(xb[t * 128:(t + 1) * 128], wk_ref[...], preferred_element_type=F32)
             for t in range(RB // 128)], axis=0)
        ka = jnp.max(jnp.abs(ks).reshape(RB // 8, 8, D), axis=0)
        kamax = ka if kamax is None else jnp.maximum(kamax, ka)
        kp = pk(ks.astype(BF16))
        for j in range(NSLAB):
            sh = 8 * j
            if j == 0:
                sl = kp[:, 0:128]
            elif j < NSLAB - 1:
                sl = pltpu.roll(jnp.where(klane >= 128 - sh, kp[:, 128 * (j - 1):128 * j],
                                          kp[:, 128 * j:128 * (j + 1)]), sh, 1)
            else:
                sl = pltpu.roll(jnp.where(klane >= 128 - sh, kp[:, 128 * (j - 1):128 * j], 0.0), sh, 1)
            k_ref[j, i * (RB // 2):(i + 1) * (RB // 2), :] = jnp.where(klane >= SLABW, ones_pk, sl)
        if i == 2:
            wqvt_ref[0:D, :] = wq_ref[...].astype(F32).T.astype(BF16)
    k2 = jnp.concatenate([kamax * kamax] * 16, axis=0)
    kn = lax.dot_general(g48, k2.astype(BF16), NT, preferred_element_type=F32)
    kmax = jnp.max(kn, axis=1, keepdims=True)

    def prep_jobs(h0, W, zt):
        jobs = []
        for par in range(2):
            h = h0 + par
            j = h // HPS
            i6 = h % HPS
            lo = i6 * DH
            for c in range(NKC):
                qi = c // 4
                part = c % 4

                def kjob(tie, c=c, par=par, j=j, lo=lo):
                    kk = tied(k_ref[j, c * HK + KM // 2:(c + 1) * HK, :], tie, zt)
                    k = pltpu.roll(upk(kk).astype(F32), (128 - lo) % 128, 1)
                    W['kb'][par][pl.ds(c * DH * PK, DH * PK), :] = jnp.concatenate(
                        [jnp.broadcast_to(k[:, d:d + 1], (PK, 128)) for d in range(DH)], axis=0)
                jobs.append((40, "k", kjob))
                for d in range(part * (DH + 1) // 4, (part + 1) * (DH + 1) // 4):
                    def qjob(tie, d=d, qi=qi, par=par, j=j, lo=lo, i6=i6):
                        r = lo + d if d < DH else SLABW + i6
                        v = jnp.broadcast_to(qt_ref[j, qi, pl.ds(r, 1), :], (8, TQ))
                        W['qb'][par][pl.ds(qi * QBR + 8 * d, 8), :] = tied(v, tie, zt)
                    jobs.append((4, "q", qjob))

                def zjob(tie, part=part, qi=qi, par=par, j=j, lo=lo, i6=i6):
                    n = 32
                    q = qt_ref[j, qi, part * n:(part + 1) * n, :]
                    qr = lax.broadcasted_iota(jnp.int32, (n, TQ), 0) + part * n
                    keep = ((qr >= lo) & (qr < lo + DH)) | (qr == SLABW + i6)
                    v = pk(jnp.where(keep, q, 0.0).astype(BF16))
                    W['qz'][pl.ds((par * NQ + qi) * 64 + part * 16, 16), :] = tied(v, tie, zt)
                jobs.append((8, "q", zjob))
        return jobs

    def views(z):
        return dict(kb=[zview(r, z) for r in kbbuf], qb=[zview(r, z) for r in qbbuf], qz=zview(qz_ref, z),
                    p=[zview(r, z) for r in pbuf])

    z0 = lax.bitcast_convert_type(k_ref[0, 0:8, :], jnp.int32) | 1
    jobs0 = prep_jobs(0, views(0), z0)
    kjobs0 = [f for _, kd, f in jobs0 if kd == "k"]
    qjobs0 = [f for _, kd, f in jobs0 if kd == "q"]
    wjobs = []
    for r in range(D // 16):
        def w1job(tie, r=r):
            w1p_ref[8 * r:8 * r + 8, :] = tied(pk(w1_ref[16 * r:16 * r + 16, :]), tie, z0)
        wjobs.append(w1job)
    for r in range(DFF // 32):
        def w2job(tie, r=r):
            w2p_ref[16 * r:16 * r + 16, :] = tied(pk(w2_ref[32 * r:32 * r + 32, :]), tie, z0)
        wjobs.append(w2job)

    for i in range(NB):
        xb = x_ref[i * RB:(i + 1) * RB, :]
        if i == 2:
            cp_wv.wait()
            cp_w[0].wait()
            cp_w[1].wait()
            cp_w[2].start()
            wqvt_ref[D:2 * D, :] = wv_ref[...].astype(F32).T.astype(BF16)
        q = lax.dot_general(wqvt_ref[0:D, :], xb, NT, preferred_element_type=F32)
        q = (q * QSCALE).astype(BF16).astype(F32)
        qn = jnp.dot(g48, (q * q).astype(BF16), preferred_element_type=F32)
        nshift = (jnp.sqrt(qn * kmax) * -0.25).astype(BF16).astype(F32)
        for j in range(NSLAB):
            nv = min(SLABW, D - SLABW * j)
            qt_ref[j, i, 0:nv] = q[SLABW * j:SLABW * j + nv]
            qt_ref[j, i, SLABW:128] = nshift[8 * j:8 * j + 8]
        for f_ in kjobs0[i * 8:(i + 1) * 8]:
            f_(None)
        if i >= 2:
            spread(wjobs[(i - 2) * 44:(i - 1) * 44], q)

    gw16 = jnp.broadcast_to(gw_ref[...].astype(F32).reshape(1, D), (16, D)).astype(BF16)
    for i in range(NB):
        cs = slice(i * RB, (i + 1) * RB)
        xb = x_ref[cs, :]
        v = lax.dot_general(jnp.concatenate([wqvt_ref[D:, :], gw16], axis=0), xb, NT, preferred_element_type=F32)
        for p in range(H // 2):
            g = v[40 * p:40 * p + 40]
            mid = g[16:24]
            vt_ref[48 * p:48 * p + 16, cs] = g[0:16]
            vt_ref[48 * p + 16:48 * p + 24, cs] = jnp.where(r8 < 4, mid, jnp.where(r8 == 4, 1.0, 0.0))
            vt_ref[48 * p + 24:48 * p + 32, cs] = jnp.where(r8 >= 4, mid, jnp.where(r8 == 0, 1.0, 0.0))
            vt_ref[48 * p + 32:48 * p + 48, cs] = g[24:40]
        grow = jax.nn.sigmoid(v[D:D + 8])
        for t in range(RB // 128):
            gb = jnp.concatenate([grow[:, 128 * t:128 * (t + 1)]] * 16, axis=0)
            g_ref[i * RB + 128 * t:i * RB + 128 * (t + 1), :] = gb.T
        if i < 3:
            spread(qjobs0[i * len(qjobs0) // 3:(i + 1) * len(qjobs0) // 3], v[0:D])

    lastacc = [None]

    def stage(h, qi, cur, par, prev, W, R, ztrue, do_a=True):
        hp, qp, orow = prev
        vrow = pl.multiple_of(hp * HP, 8)
        acc = None
        wbase = (cur % 2) * NPER * HK
        rbase = ((cur + 1) % 2) * NPER * HK
        if do_a:
            j = h // HPS
        for c in range(NKC):
            vt = vt_ref[pl.ds(vrow, HP), c * KC:(c + 1) * KC]
            pw = R['p'][c % NP][pl.ds(rbase + (c // NP) * HK, HK), :]
            d = jnp.dot(vt, upk(pw), preferred_element_type=F32)
            if acc is None:
                acc = d if lastacc[0] is None else jnp.where(ztrue, d, lastacc[0])
            else:
                acc = acc + d
            if not do_a:
                continue
            s = jnp.dot(upk(k_ref[j, c * HK:c * HK + KM // 2, :]), upk(R['qz'][pl.ds(cur * 64, 64), :]),
                        preferred_element_type=F32)
            W['p'][c % NP][pl.ds(wbase + (c // NP) * HK, KM // 2), :] = pk(jnp.exp2(s).astype(BF16))
            tprev = None
            for g in range(NG):
                kb = R['kb'][par][pl.ds(c * DH * PK, DH * PK), :]
                kb = jnp.concatenate([kb] * (GW // 128), axis=1)
                qb = R['qb'][par][pl.ds(qi * QBR, QBR), g * GW:(g + 1) * GW].reshape(DH + 1, 8, GW)
                qb = jnp.concatenate([qb] * (PK // 8), axis=1).reshape((DH + 1) * PK, GW)
                t = qb[DH * PK:]
                if tprev is not None:
                    t = jnp.where(ztrue, t, tprev)
                for dd in range(DH):
                    t = t + kb[dd * PK:(dd + 1) * PK] * qb[dd * PK:(dd + 1) * PK]
                W['p'][c % NP][pl.ds(wbase + (c // NP) * HK + KM // 2, PK // 2), g * GW:(g + 1) * GW] = pk(
                    jnp.exp2(t).astype(BF16))
                tprev = t
        ot_ref[pl.ds(pl.multiple_of(orow, 8), HP), qp * TQ:(qp + 1) * TQ] = acc
        lastacc[0] = acc

    def body(u, carry):
        z = lax.shift_right_logical(u, 8)
        z2 = lax.shift_right_logical(u, 9)
        W = views(z)
        R = views(z2)
        ztrue = z2 == 0
        lastacc[0] = None
        for i in range(U):
            h = 2 * u + i // NQ
            qi = i % NQ
            if i == 0:
                hp = jnp.maximum(2 * u - 1, 0)
                prev = (hp, NQ - 1, jnp.where(u == 0, H * HP, hp * HP))
            else:
                hp = 2 * u + (i - 1) // NQ
                prev = (hp, (i - 1) % NQ, hp * HP)
            stage(h, qi, i, (i // NQ) % 2, prev, W, R, ztrue)

        rs = pl.ds(pl.multiple_of(u * FR, FR), FR)
        xb = x_ref[rs, :]
        jobs = prep_jobs(jnp.minimum(2 * u + 2, H - 2), W, z)
        tot = sum(jb[0] for jb in jobs)
        durs = [640, 640] + [128] * 14
        cum = [sum(durs[:i + 1]) / sum(durs) for i in range(len(durs))]
        state = dict(i=0, acc=0)

        def release(k, val):
            nr = val.shape[0] // 8
            nv = nr * (val.shape[1] // 128)
            while state["i"] < len(jobs) and (state["acc"] + jobs[state["i"]][0] / 2) / tot <= cum[k]:
                cst, _, fn = jobs[state["i"]]
                lo_ = cum[k - 1] if k else 0.0
                frac = min(max((state["acc"] / tot - lo_) / (cum[k] - lo_), 0.0), 0.999)
                col, row = divmod(int(frac * nv), nr)
                fn(val[8 * row:8 * row + 8, 128 * col:128 * (col + 1)])
                state["i"] += 1
                state["acc"] += cst
        hs = []
        for n in range(3):
            w = w1p_ref[:, 512 * n:512 * (n + 1)]
            rows = [w[64 * t:64 * (t + 1)] for t in range(5)]
            for (t, a_) in {0: [(4, 0)], 1: [(0, 1), (2, 2), (4, 3)]}.get(n, []):
                top = jnp.where(ztrue, rows[t][0:8], R['p'][a_][0:8, :])
                rows[t] = jnp.concatenate([top, rows[t][8:]], axis=0)
            w = jnp.concatenate(rows, axis=0)
            hf = jnp.maximum(jnp.dot(xb, upk(w), preferred_element_type=F32), 0.0)
            release(n, hf)
            hs.append(hf.astype(BF16))
        g1 = 1.0 - g_ref[rs, :]
        for n in range(5):
            bn = None
            for kk in range(3):
                pd = jnp.dot(hs[kk], upk(w2p_ref[256 * kk:256 * (kk + 1), 128 * n:128 * (n + 1)]),
                             preferred_element_type=F32)
                bn = pd if bn is None else bn + pd
                if 3 + n * 3 + kk < len(durs):
                    release(3 + n * 3 + kk, pd)
            bm_ref[rs, 128 * n:128 * (n + 1)] = g1 * bn
        assert state["i"] == len(jobs)
        return carry
    lax.fori_loop(0, NIT, body, 0)
    lastacc[0] = None
    stage(0, 0, 0, 0, (H - 1, NQ - 1, (H - 1) * HP), None, views(0), None, do_a=False)

    cp_w[2].wait()

    def rows_of(i):
        return pl.ds(i * FB, FB) if isinstance(i, int) else pl.ds(pl.multiple_of(i * FB, FB), FB)

    def out_cp(i):
        return pltpu.make_async_copy(out_ref.at[rows_of(i)], out_hbm.at[rows_of(i)], sem_out.at[i])

    r8f = lax.broadcasted_iota(jnp.int32, (8, FB), 0)

    def fin(i, check):
        rs = rows_of(i)
        parts = []
        lmin = amax = None
        for p in range(H // 2):
            e = ot_ref[48 * p:48 * p + 24, rs]
            o = ot_ref[48 * p + 24:48 * p + 48, rs]
            if check:
                l = jnp.where(r8f < 4, o[0:8], e[16:24])
                lmin = l if lmin is None else jnp.minimum(lmin, l)
                for t_ in (e, o):
                    am = jnp.max(jnp.abs(t_).reshape(3, 8, FB), axis=0)
                    amax = am if amax is None else jnp.maximum(amax, am)
            e = e * (1.0 / e[DH:DH + 1])
            o = o * (1.0 / o[0:1])
            parts += [e[0:16], jnp.where(r8f < 4, e[16:24], o[0:8]), o[8:24]]
        ot = jnp.concatenate(parts, axis=0).astype(BF16)
        a = lax.dot_general(ot, wo_ref[...], TN, preferred_element_type=F32)
        g = jnp.concatenate([g_ref[rs, :]] * (D // 128), axis=1)
        out_ref[rs, :] = (g * a + bm_ref[rs, :]).astype(out_ref.dtype)
        out_cp(i).start()
        if check:
            ok = ((lmin >= 2.0 ** -60) | ((r8f != 0) & (r8f != 4))) & (amax <= 2.0 ** 120)
            return jnp.where(ok, 0.0, 1.0)

    bad = None
    for i in range(NFB):
        bi = fin(i, True)
        bad = bi if bad is None else jnp.maximum(bad, bi)
    nbad = jnp.max(jnp.max(bad, axis=1, keepdims=True), axis=0, keepdims=True)[0, 0]
    for i in range(NFB):
        out_cp(i).wait()

    @pl.when(nbad > FORCE)
    def _():
        qrow = lax.broadcasted_iota(jnp.int32, (128, TQ), 0)

        def fb(t, c):
            h = t // NQ
            qi = t % NQ
            j = h // HPS
            lo = (h % HPS) * DH
            qz = jnp.where((qrow >= lo) & (qrow < lo + DH), qt_ref[j, qi], 0.0).astype(BF16)
            s = jnp.dot(upk(k_ref[j]), qz, preferred_element_type=F32)
            m = jnp.max(s, axis=0, keepdims=True)
            p = jnp.exp2(s - m).astype(BF16)
            vrow = pl.multiple_of(h * HP, 8)
            acc = jnp.dot(vt_ref[pl.ds(vrow, HP), :], p, preferred_element_type=F32)
            ot_ref[pl.ds(vrow, HP), pl.ds(pl.multiple_of(qi * TQ, TQ), TQ)] = acc
            return c
        lax.fori_loop(0, NSTEP, fb, 0)

        def fin2(i, c):
            fin(i, False)
            out_cp(i).wait()
            return c
        lax.fori_loop(0, NFB, fin2, 0)


FORCE = 0.0

_SCRATCH = [
    pltpu.VMEM((S, D), BF16),
    pltpu.VMEM((D, D), BF16),
    pltpu.VMEM((D, D), BF16),
    pltpu.VMEM((D, D), BF16),
    pltpu.VMEM((D, D), BF16),
    pltpu.VMEM((D, DFF), BF16),
    pltpu.VMEM((DFF, D), BF16),
    pltpu.VMEM((S, D), BF16),
    pltpu.VMEM((2 * D, D), BF16),
    pltpu.VMEM((D // 2, DFF), F32),
    pltpu.VMEM((DFF // 2, D), F32),
    pltpu.VMEM((NSLAB, S // 2, 128), F32),
    pltpu.VMEM((NSLAB, NQ, 128, TQ), F32),
    pltpu.VMEM((H * HP, S), F32),
    pltpu.VMEM((H * HP + HP, S), F32),
    pltpu.VMEM((S, D), F32),
    pltpu.VMEM((S, 128), F32),
    pltpu.VMEM((U * 64, TQ), F32),
    pltpu.VMEM((NQ * QBR, TQ), F32),
    pltpu.VMEM((NQ * QBR, TQ), F32),
    pltpu.VMEM((DH * NKC * PK, 128), F32),
    pltpu.VMEM((DH * NKC * PK, 128), F32),
] + [pltpu.VMEM((2 * NPER * HK, TQ), F32)] * NP + [
    pltpu.SemaphoreType.DMA((6,)),
    pltpu.SemaphoreType.DMA((NB,)),
    pltpu.SemaphoreType.DMA((NFB,)),
]


@jax.jit
def pallas_gated_mix__softmax_full_mha__dense_activation_relu__prompt_kernel(
    A_x: jax.Array,
    A_wqkv: jax.Array,
    A_wo: jax.Array,
    B_x: jax.Array,
    B_w1: jax.Array,
    B_w2: jax.Array,
    gate_w: jax.Array,
):
    anyspec = pl.BlockSpec(memory_space=pl.ANY)
    out = pl.pallas_call(
        _kernel,
        out_shape=jax.ShapeDtypeStruct((S, D), BF16),
        in_specs=[anyspec] * 5 + [pl.BlockSpec(memory_space=pltpu.VMEM)],
        out_specs=anyspec,
        scratch_shapes=_SCRATCH,
        compiler_params=pltpu.CompilerParams(vmem_limit_bytes=100 * 1024 * 1024),
    )(A_x.reshape(S, D), A_wqkv, A_wo, B_w1, B_w2, gate_w)
    return out.reshape(1, S, D)
```

```python
import math

import jax
import jax.numpy as jnp
from jax import lax
import jax.experimental.pallas as pl
import jax.experimental.pallas.tpu as pltpu

S, D, H, DH, DFF = 2048, 640, 32, 20, 1536
HP = 24
HPS = 6
NSLAB = 6
SLABW = HPS * DH
F32 = jnp.float32
BF16 = jnp.bfloat16

TQ = 512
KC = 128
PK = 16
NP = 4
NG = 2
FB = 128
RB = TQ
NB = S // RB
NQ = S // TQ
NFB = S // FB
NSTEP = H * NQ
NKC = S // KC
NPER = NKC // NP
HK = KC // 2
KM = KC - PK
U = 2 * NQ
NIT = NSTEP // U
FR = S // NIT
QBR = (DH + 1) * 8
GW = TQ // NG
QSCALE = (DH ** -0.5) * math.log2(math.e)

NT = (((1,), (1,)), ((), ()))


def pk(x):
    return pltpu.bitcast(x, F32)


def upk(x):
    return pltpu.bitcast(x, BF16)


def zview(ref, z):
    if isinstance(z, int):
        return ref
    return ref.at[pl.ds(pl.multiple_of(z * 8, 8), ref.shape[0])]


def tied(v, tie, zt):
    if tie is None:
        return v
    t = jnp.concatenate([tie] * (v.shape[1] // 128), axis=1)
    t = jnp.concatenate([t] * (v.shape[0] // 8), axis=0)
    if zt.ndim:
        m = jnp.concatenate([zt] * (v.shape[1] // 128), axis=1)
        m = jnp.concatenate([m] * (v.shape[0] // 8), axis=0)
        return jnp.where(m != 0, v, t)
    return jnp.where(zt == 0, v, t)


def spread(fns, val):
    nr = val.shape[0] // 8
    nv = nr * (val.shape[1] // 128)
    for n_, fn in enumerate(fns):
        col, row = divmod((n_ * nv) // len(fns), nr)
        fn(val[8 * row:8 * row + 8, 128 * col:128 * (col + 1)])


def _kernel(x_hbm, wqkv_hbm, wo_hbm, w1_hbm, w2_hbm, gw_ref, out_hbm,
            x_ref, wq_ref, wk_ref, wv_ref, wo_ref, w1_ref, w2_ref, out_ref,
            wqvt_ref, w1p_ref, w2p_ref, k_ref, qt_ref, vt_ref, ot_ref, bm_ref, g_ref,
            qz_ref, qb0_ref, qb1_ref, kb0_ref, kb1_ref, p0, p1, p2, p3,
            sem_in, sem_x, sem_out):
    kbbuf = (kb0_ref, kb1_ref)
    qbbuf = (qb0_ref, qb1_ref)
    pbuf = (p0, p1, p2, p3)

    cp_wk = pltpu.make_async_copy(wqkv_hbm.at[:, D:2 * D], wk_ref, sem_in.at[0])
    cp_wq = pltpu.make_async_copy(wqkv_hbm.at[:, 0:D], wq_ref, sem_in.at[1])
    cp_wv = pltpu.make_async_copy(wqkv_hbm.at[:, 2 * D:3 * D], wv_ref, sem_in.at[2])
    cp_x = [pltpu.make_async_copy(x_hbm.at[i * RB:(i + 1) * RB], x_ref.at[i * RB:(i + 1) * RB], sem_x.at[i])
            for i in range(NB)]
    cp_w = [pltpu.make_async_copy(a, b, sem_in.at[3 + n])
            for n, (a, b) in enumerate(((w1_hbm, w1_ref), (w2_hbm, w2_ref), (wo_hbm, wo_ref)))]
    cp_wk.start()
    cp_x[0].start()
    for pb in pbuf:
        pb[NPER * HK:2 * NPER * HK, :] = jnp.zeros((NPER * HK, TQ), F32)
    for i in range(NQ):
        qt_ref[NSLAB - 1, i, 40:120] = jnp.zeros((80, TQ), F32)
    cp_wk.wait()
    cp_x[1].start()

    klane = lax.broadcasted_iota(jnp.int32, (RB // 2, 128), 1)
    ones_pk = pk(jnp.where(lax.broadcasted_iota(jnp.int32, (RB, 128), 1) < SLABW + HPS, 1.0, 0.0).astype(BF16))
    g48r = lax.broadcasted_iota(jnp.int32, (8 * NSLAB, D), 0)
    g48c = lax.broadcasted_iota(jnp.int32, (8 * NSLAB, D), 1)
    g48h = (g48r // 8) * HPS + (g48r % 8)
    g48 = jnp.where((g48c >= g48h * DH) & (g48c < g48h * DH + DH) & (g48r % 8 < HPS), 1.0, 0.0).astype(BF16)
    r8 = lax.broadcasted_iota(jnp.int32, (8, RB), 0)

    kamax = None
    for i in range(NB):
        if i == 0:
            cp_x[0].wait()
            cp_x[2].start()
            cp_x[3].start()
        if i == 1:
            cp_x[1].wait()
            cp_wq.start()
        if i == 2:
            cp_x[2].wait()
            cp_x[3].wait()
            cp_wq.wait()
            cp_wv.start()
            cp_w[0].start()
            cp_w[1].start()
        xb = x_ref[i * RB:(i + 1) * RB, :]
        ks = jnp.concatenate(
            [jnp.dot(xb[t * 128:(t + 1) * 128], wk_ref[...], preferred_element_type=F32)
             for t in range(RB // 128)], axis=0)
        ka = jnp.max(jnp.abs(ks).reshape(RB // 8, 8, D), axis=0)
        kamax = ka if kamax is None else jnp.maximum(kamax, ka)
        kp = pk(ks.astype(BF16))
        for j in range(NSLAB):
            sh = 8 * j
            if j == 0:
                sl = kp[:, 0:128]
            elif j < NSLAB - 1:
                sl = pltpu.roll(jnp.where(klane >= 128 - sh, kp[:, 128 * (j - 1):128 * j],
                                          kp[:, 128 * j:128 * (j + 1)]), sh, 1)
            else:
                sl = pltpu.roll(jnp.where(klane >= 128 - sh, kp[:, 128 * (j - 1):128 * j], 0.0), sh, 1)
            k_ref[j, i * (RB // 2):(i + 1) * (RB // 2), :] = jnp.where(klane >= SLABW, ones_pk, sl)
        if i == 2:
            wqvt_ref[0:D, :] = wq_ref[...].astype(F32).T.astype(BF16)
    k2 = jnp.concatenate([kamax * kamax] * 16, axis=0)
    kn = lax.dot_general(g48, k2.astype(BF16), NT, preferred_element_type=F32)
    kmax = jnp.max(kn, axis=1, keepdims=True)

    def prep_jobs(h0, W, zt):
        jobs = []
        for par in range(2):
            h = h0 + par
            j = h // HPS
            i6 = h % HPS
            lo = i6 * DH
            for c in range(NKC):
                qi = c // 4
                part = c % 4

                def kjob(tie, c=c, par=par, j=j, lo=lo):
                    kk = tied(k_ref[j, c * HK + KM // 2:(c + 1) * HK, :], tie, zt)
                    k = pltpu.roll(upk(kk).astype(F32), (128 - lo) % 128, 1)
                    W['kb'][par][pl.ds(c * DH * PK, DH * PK), :] = jnp.concatenate(
                        [jnp.broadcast_to(k[:, d:d + 1], (PK, 128)) for d in range(DH)], axis=0)
                jobs.append((40, "k", kjob))
                for d in range(part * (DH + 1) // 4, (part + 1) * (DH + 1) // 4):
                    def qjob(tie, d=d, qi=qi, par=par, j=j, lo=lo, i6=i6):
                        r = lo + d if d < DH else SLABW + i6
                        v = jnp.broadcast_to(qt_ref[j, qi, pl.ds(r, 1), :], (8, TQ))
                        W['qb'][par][pl.ds(qi * QBR + 8 * d, 8), :] = tied(v, tie, zt)
                    jobs.append((4, "q", qjob))

                def zjob(tie, part=part, qi=qi, par=par, j=j, lo=lo, i6=i6):
                    n = 32
                    q = qt_ref[j, qi, part * n:(part + 1) * n, :]
                    qr = lax.broadcasted_iota(jnp.int32, (n, TQ), 0) + part * n
                    keep = ((qr >= lo) & (qr < lo + DH)) | (qr == SLABW + i6)
                    v = pk(jnp.where(keep, q, 0.0).astype(BF16))
                    W['qz'][pl.ds((par * NQ + qi) * 64 + part * 16, 16), :] = tied(v, tie, zt)
                jobs.append((8, "q", zjob))
        return jobs

    def views(z):
        return dict(kb=[zview(r, z) for r in kbbuf], qb=[zview(r, z) for r in qbbuf], qz=zview(qz_ref, z),
                    p=[zview(r, z) for r in pbuf])

    z0 = lax.bitcast_convert_type(k_ref[0, 0:8, :], jnp.int32) | 1
    jobs0 = prep_jobs(0, views(0), z0)
    kjobs0 = [f for _, kd, f in jobs0 if kd == "k"]
    qjobs0 = [f for _, kd, f in jobs0 if kd == "q"]
    wjobs = []
    for r in range(D // 16):
        def w1job(tie, r=r):
            w1p_ref[8 * r:8 * r + 8, :] = tied(pk(w1_ref[16 * r:16 * r + 16, :]), tie, z0)
        wjobs.append(w1job)
    for r in range(DFF // 32):
        def w2job(tie, r=r):
            w2p_ref[16 * r:16 * r + 16, :] = tied(pk(w2_ref[32 * r:32 * r + 32, :]), tie, z0)
        wjobs.append(w2job)

    for i in range(NB):
        xb = x_ref[i * RB:(i + 1) * RB, :]
        if i == 2:
            cp_wv.wait()
            cp_w[0].wait()
            cp_w[1].wait()
            cp_w[2].start()
            wqvt_ref[D:2 * D, :] = wv_ref[...].astype(F32).T.astype(BF16)
        q = lax.dot_general(wqvt_ref[0:D, :], xb, NT, preferred_element_type=F32)
        q = (q * QSCALE).astype(BF16).astype(F32)
        qn = jnp.dot(g48, (q * q).astype(BF16), preferred_element_type=F32)
        nshift = (jnp.sqrt(qn * kmax) * -0.25).astype(BF16).astype(F32)
        for j in range(NSLAB):
            nv = min(SLABW, D - SLABW * j)
            qt_ref[j, i, 0:nv] = q[SLABW * j:SLABW * j + nv]
            qt_ref[j, i, SLABW:128] = nshift[8 * j:8 * j + 8]
        for f_ in kjobs0[i * 8:(i + 1) * 8]:
            f_(None)
        if i >= 2:
            spread(wjobs[(i - 2) * 44:(i - 1) * 44], q)

    gw16 = jnp.broadcast_to(gw_ref[...].astype(F32).reshape(1, D), (16, D)).astype(BF16)
    for i in range(NB):
        cs = slice(i * RB, (i + 1) * RB)
        xb = x_ref[cs, :]
        v = lax.dot_general(jnp.concatenate([wqvt_ref[D:, :], gw16], axis=0), xb, NT, preferred_element_type=F32)
        for p in range(H // 2):
            g = v[40 * p:40 * p + 40]
            mid = g[16:24]
            vt_ref[48 * p:48 * p + 16, cs] = g[0:16]
            vt_ref[48 * p + 16:48 * p + 24, cs] = jnp.where(r8 < 4, mid, jnp.where(r8 == 4, 1.0, 0.0))
            vt_ref[48 * p + 24:48 * p + 32, cs] = jnp.where(r8 >= 4, mid, jnp.where(r8 == 0, 1.0, 0.0))
            vt_ref[48 * p + 32:48 * p + 48, cs] = g[24:40]
        grow = jax.nn.sigmoid(v[D:D + 8])
        for t in range(RB // 128):
            gb = jnp.concatenate([grow[:, 128 * t:128 * (t + 1)]] * 16, axis=0)
            g_ref[i * RB + 128 * t:i * RB + 128 * (t + 1), :] = gb.T
        if i < 3:
            spread(qjobs0[i * len(qjobs0) // 3:(i + 1) * len(qjobs0) // 3], v[0:D])

    lastacc = [None]

    def stage(h, qi, cur, par, prev, W, R, ztrue, do_a=True):
        hp, qp, orow = prev
        vrow = pl.multiple_of(hp * HP, 8)
        acc = None
        wbase = (cur % 2) * NPER * HK
        rbase = ((cur + 1) % 2) * NPER * HK
        if do_a:
            j = h // HPS
        for c in range(NKC):
            vt = vt_ref[pl.ds(vrow, HP), c * KC:(c + 1) * KC]
            pw = R['p'][c % NP][pl.ds(rbase + (c // NP) * HK, HK), :]
            d = jnp.dot(vt, upk(pw), preferred_element_type=F32)
            if acc is None:
                acc = d if lastacc[0] is None else jnp.where(ztrue, d, lastacc[0])
            else:
                acc = acc + d
            if not do_a:
                continue
            s = jnp.dot(upk(k_ref[j, c * HK:c * HK + KM // 2, :]), upk(R['qz'][pl.ds(cur * 64, 64), :]),
                        preferred_element_type=F32)
            W['p'][c % NP][pl.ds(wbase + (c // NP) * HK, KM // 2), :] = pk(jnp.exp2(s).astype(BF16))
            tprev = None
            for g in range(NG):
                kb = R['kb'][par][pl.ds(c * DH * PK, DH * PK), :]
                kb = jnp.concatenate([kb] * (GW // 128), axis=1)
                qb = R['qb'][par][pl.ds(qi * QBR, QBR), g * GW:(g + 1) * GW].reshape(DH + 1, 8, GW)
                qb = jnp.concatenate([qb] * (PK // 8), axis=1).reshape((DH + 1) * PK, GW)
                t = qb[DH * PK:]
                if tprev is not None:
                    t = jnp.where(ztrue, t, tprev)
                for dd in range(DH):
                    t = t + kb[dd * PK:(dd + 1) * PK] * qb[dd * PK:(dd + 1) * PK]
                W['p'][c % NP][pl.ds(wbase + (c // NP) * HK + KM // 2, PK // 2), g * GW:(g + 1) * GW] = pk(
                    jnp.exp2(t).astype(BF16))
                tprev = t
        ot_ref[pl.ds(pl.multiple_of(orow, 8), HP), qp * TQ:(qp + 1) * TQ] = acc
        lastacc[0] = acc

    def body(u, carry):
        z = lax.shift_right_logical(u, 8)
        z2 = lax.shift_right_logical(u, 9)
        W = views(z)
        R = views(z2)
        ztrue = z2 == 0
        lastacc[0] = None
        for i in range(U):
            h = 2 * u + i // NQ
            qi = i % NQ
            if i == 0:
                hp = jnp.maximum(2 * u - 1, 0)
                prev = (hp, NQ - 1, jnp.where(u == 0, H * HP, hp * HP))
            else:
                hp = 2 * u + (i - 1) // NQ
                prev = (hp, (i - 1) % NQ, hp * HP)
            stage(h, qi, i, (i // NQ) % 2, prev, W, R, ztrue)

        rs = pl.ds(pl.multiple_of(u * FR, FR), FR)
        xb = x_ref[rs, :]
        jobs = prep_jobs(jnp.minimum(2 * u + 2, H - 2), W, z)
        tot = sum(jb[0] for jb in jobs)
        durs = [640, 640] + [128] * 14
        cum = [sum(durs[:i + 1]) / sum(durs) for i in range(len(durs))]
        state = dict(i=0, acc=0)

        def release(k, val):
            nr = val.shape[0] // 8
            nv = nr * (val.shape[1] // 128)
            while state["i"] < len(jobs) and (state["acc"] + jobs[state["i"]][0] / 2) / tot <= cum[k]:
                cst, _, fn = jobs[state["i"]]
                lo_ = cum[k - 1] if k else 0.0
                frac = min(max((state["acc"] / tot - lo_) / (cum[k] - lo_), 0.0), 0.999)
                col, row = divmod(int(frac * nv), nr)
                fn(val[8 * row:8 * row + 8, 128 * col:128 * (col + 1)])
                state["i"] += 1
                state["acc"] += cst
        hs = []
        for n in range(3):
            w = w1p_ref[:, 512 * n:512 * (n + 1)]
            rows = [w[64 * t:64 * (t + 1)] for t in range(5)]
            for (t, a_) in {0: [(4, 0)], 1: [(0, 1), (2, 2), (4, 3)]}.get(n, []):
                top = jnp.where(ztrue, rows[t][0:8], R['p'][a_][0:8, :])
                rows[t] = jnp.concatenate([top, rows[t][8:]], axis=0)
            w = jnp.concatenate(rows, axis=0)
            hf = jnp.maximum(jnp.dot(xb, upk(w), preferred_element_type=F32), 0.0)
            release(n, hf)
            hs.append(hf.astype(BF16))
        g1 = 1.0 - g_ref[rs, :]
        for n in range(5):
            bn = None
            for kk in range(3):
                pd = jnp.dot(hs[kk], upk(w2p_ref[256 * kk:256 * (kk + 1), 128 * n:128 * (n + 1)]),
                             preferred_element_type=F32)
                bn = pd if bn is None else bn + pd
                if 3 + n * 3 + kk < len(durs):
                    release(3 + n * 3 + kk, pd)
            bm_ref[rs, 128 * n:128 * (n + 1)] = g1 * bn
        assert state["i"] == len(jobs)
        return carry
    lax.fori_loop(0, NIT, body, 0)
    lastacc[0] = None
    stage(0, 0, 0, 0, (H - 1, NQ - 1, (H - 1) * HP), None, views(0), None, do_a=False)

    cp_w[2].wait()

    def rows_of(i):
        return pl.ds(i * FB, FB) if isinstance(i, int) else pl.ds(pl.multiple_of(i * FB, FB), FB)

    def out_cp(i):
        return pltpu.make_async_copy(out_ref.at[rows_of(i)], out_hbm.at[rows_of(i)], sem_out.at[i])

    r8f = lax.broadcasted_iota(jnp.int32, (8, FB), 0)

    def fin(i, check):
        rs = rows_of(i)
        parts = []
        lmin = amax = None
        for p in range(H // 2):
            e = ot_ref[48 * p:48 * p + 24, rs]
            o = ot_ref[48 * p + 24:48 * p + 48, rs]
            if check:
                l = jnp.where(r8f < 4, o[0:8], e[16:24])
                lmin = l if lmin is None else jnp.minimum(lmin, l)
                for t_ in (e, o):
                    am = jnp.max(jnp.abs(t_).reshape(3, 8, FB), axis=0)
                    amax = am if amax is None else jnp.maximum(amax, am)
            e = e * (1.0 / e[DH:DH + 1])
            o = o * (1.0 / o[0:1])
            parts += [e[0:16], jnp.where(r8f < 4, e[16:24], o[0:8]), o[8:24]]
        ot = jnp.concatenate(parts, axis=0).T.astype(BF16)
        a = jnp.dot(ot, wo_ref[...], preferred_element_type=F32)
        g = jnp.concatenate([g_ref[rs, :]] * (D // 128), axis=1)
        out_ref[rs, :] = (g * a + bm_ref[rs, :]).astype(out_ref.dtype)
        out_cp(i).start()
        if check:
            ok = ((lmin >= 2.0 ** -60) | ((r8f != 0) & (r8f != 4))) & (amax <= 2.0 ** 120)
            return jnp.where(ok, 0.0, 1.0)

    bad = None
    for i in range(NFB):
        bi = fin(i, True)
        bad = bi if bad is None else jnp.maximum(bad, bi)
    nbad = jnp.max(jnp.max(bad, axis=1, keepdims=True), axis=0, keepdims=True)[0, 0]
    for i in range(NFB):
        out_cp(i).wait()

    @pl.when(nbad > 0.0)
    def _():
        qrow = lax.broadcasted_iota(jnp.int32, (128, TQ), 0)

        def fb(t, c):
            h = t // NQ
            qi = t % NQ
            j = h // HPS
            lo = (h % HPS) * DH
            qz = jnp.where((qrow >= lo) & (qrow < lo + DH), qt_ref[j, qi], 0.0).astype(BF16)
            s = jnp.dot(upk(k_ref[j]), qz, preferred_element_type=F32)
            m = jnp.max(s, axis=0, keepdims=True)
            p = jnp.exp2(s - m).astype(BF16)
            vrow = pl.multiple_of(h * HP, 8)
            acc = jnp.dot(vt_ref[pl.ds(vrow, HP), :], p, preferred_element_type=F32)
            ot_ref[pl.ds(vrow, HP), pl.ds(pl.multiple_of(qi * TQ, TQ), TQ)] = acc
            return c
        lax.fori_loop(0, NSTEP, fb, 0)

        def fin2(i, c):
            fin(i, False)
            out_cp(i).wait()
            return c
        lax.fori_loop(0, NFB, fin2, 0)


_SCRATCH = [
    pltpu.VMEM((S, D), BF16),
    pltpu.VMEM((D, D), BF16),
    pltpu.VMEM((D, D), BF16),
    pltpu.VMEM((D, D), BF16),
    pltpu.VMEM((D, D), BF16),
    pltpu.VMEM((D, DFF), BF16),
    pltpu.VMEM((DFF, D), BF16),
    pltpu.VMEM((S, D), BF16),
    pltpu.VMEM((2 * D, D), BF16),
    pltpu.VMEM((D // 2, DFF), F32),
    pltpu.VMEM((DFF // 2, D), F32),
    pltpu.VMEM((NSLAB, S // 2, 128), F32),
    pltpu.VMEM((NSLAB, NQ, 128, TQ), F32),
    pltpu.VMEM((H * HP, S), F32),
    pltpu.VMEM((H * HP + HP, S), F32),
    pltpu.VMEM((S, D), F32),
    pltpu.VMEM((S, 128), F32),
    pltpu.VMEM((U * 64, TQ), F32),
    pltpu.VMEM((NQ * QBR, TQ), F32),
    pltpu.VMEM((NQ * QBR, TQ), F32),
    pltpu.VMEM((DH * NKC * PK, 128), F32),
    pltpu.VMEM((DH * NKC * PK, 128), F32),
] + [pltpu.VMEM((2 * NPER * HK, TQ), F32)] * NP + [
    pltpu.SemaphoreType.DMA((6,)),
    pltpu.SemaphoreType.DMA((NB,)),
    pltpu.SemaphoreType.DMA((NFB,)),
]


@jax.jit
def pallas_gated_mix__softmax_full_mha__dense_activation_relu__prompt_kernel(
    A_x: jax.Array,
    A_wqkv: jax.Array,
    A_wo: jax.Array,
    B_x: jax.Array,
    B_w1: jax.Array,
    B_w2: jax.Array,
    gate_w: jax.Array,
):
    anyspec = pl.BlockSpec(memory_space=pl.ANY)
    out = pl.pallas_call(
        _kernel,
        out_shape=jax.ShapeDtypeStruct((S, D), BF16),
        in_specs=[anyspec] * 5 + [pl.BlockSpec(memory_space=pltpu.VMEM)],
        out_specs=anyspec,
        scratch_shapes=_SCRATCH,
        compiler_params=pltpu.CompilerParams(vmem_limit_bytes=100 * 1024 * 1024),
    )(A_x.reshape(S, D), A_wqkv, A_wo, B_w1, B_w2, gate_w)
    return out.reshape(1, S, D)
```

```python
import math

import jax
import jax.numpy as jnp
from jax import lax
import jax.experimental.pallas as pl
import jax.experimental.pallas.tpu as pltpu

S, D, H, DH, DFF = 2048, 640, 32, 20, 1536
HP = 24
HPS = 6
NSLAB = 6
SLABW = HPS * DH
NT5 = D // 128
F32 = jnp.float32
BF16 = jnp.bfloat16
I32 = jnp.int32
I8 = jnp.int8

TQ = 512
KC = 512
NP = 2
FB = 128
RB = TQ
NB = S // RB
NQ = S // TQ
NFB = S // FB
NSTEP = H * NQ
NKC = S // KC
NPER = NKC // NP
HK = KC // 2
U = 2 * NQ
NIT = NSTEP // U
FR = S // NIT
QSCALE = (DH ** -0.5) * math.log2(math.e)
YMAX = 378.0
NLIMB = 5
NSH = 128 - NLIMB * DH

NT = (((1,), (1,)), ((), ()))


def pk(x):
    return pltpu.bitcast(x, F32)


def upk(x):
    return pltpu.bitcast(x, BF16)


def pk8(x):
    return pltpu.bitcast(x.astype(I8), I32)


def up8(x):
    return pltpu.bitcast(x, I8)


def iround(x):
    return jnp.round(x).astype(I32)


def zview(ref, z):
    if isinstance(z, int):
        return ref
    return ref.at[pl.ds(pl.multiple_of(z * 8, 8), ref.shape[0])]


def tied(v, tie, zt):
    if tie is None:
        return v
    if tie.dtype != v.dtype:
        tie = lax.bitcast_convert_type(tie, v.dtype)
    t = jnp.concatenate([tie] * (v.shape[1] // 128), axis=1)
    t = jnp.concatenate([t] * (v.shape[0] // 8), axis=0)
    if zt.ndim:
        m = jnp.concatenate([zt] * (v.shape[1] // 128), axis=1)
        m = jnp.concatenate([m] * (v.shape[0] // 8), axis=0)
        return jnp.where(m != 0, v, t)
    return jnp.where(zt == 0, v, t)


def spread(fns, val):
    nr = val.shape[0] // 8
    nv = nr * (val.shape[1] // 128)
    for n_, fn in enumerate(fns):
        col, row = divmod((n_ * nv) // len(fns), nr)
        fn(val[8 * row:8 * row + 8, 128 * col:128 * (col + 1)])


def _kernel(x_hbm, wqkv_hbm, wo_hbm, w1_hbm, w2_hbm, gw_ref, out_hbm,
            x_ref, wq_ref, wk_ref, wv_ref, wo_ref, w1_ref, w2_ref, out_ref,
            wqvt_ref, w1p_ref, w2p_ref, kf_ref, r8_ref, qt_ref, vt_ref, ot_ref, bm_ref, g_ref,
            k8_ref, qz_ref, fq_ref, *rest):
    pbuf = rest[:NP]
    sem_in, sem_x, sem_out = rest[NP:]

    cp_wk = pltpu.make_async_copy(wqkv_hbm.at[:, D:2 * D], wk_ref, sem_in.at[0])
    cp_wq = pltpu.make_async_copy(wqkv_hbm.at[:, 0:D], wq_ref, sem_in.at[1])
    cp_wv = pltpu.make_async_copy(wqkv_hbm.at[:, 2 * D:3 * D], wv_ref, sem_in.at[2])
    cp_x = [pltpu.make_async_copy(x_hbm.at[i * RB:(i + 1) * RB], x_ref.at[i * RB:(i + 1) * RB], sem_x.at[i])
            for i in range(NB)]
    cp_w = [pltpu.make_async_copy(a, b, sem_in.at[3 + n])
            for n, (a, b) in enumerate(((w1_hbm, w1_ref), (w2_hbm, w2_ref), (wo_hbm, wo_ref)))]
    cp_wk.start()
    cp_x[0].start()
    for pb in pbuf:
        pb[NPER * HK:2 * NPER * HK, :] = jnp.zeros((NPER * HK, TQ), F32)
    cp_wk.wait()
    cp_x[1].start()
    r8 = lax.broadcasted_iota(I32, (8, RB), 0)

    kamax = ksq = None
    for i in range(NB):
        if i == 0:
            cp_x[0].wait()
            cp_x[2].start()
            cp_x[3].start()
        if i == 1:
            cp_x[1].wait()
            cp_wq.start()
        if i == 2:
            cp_x[2].wait()
            cp_x[3].wait()
            cp_wq.wait()
            cp_wv.start()
            cp_w[0].start()
            cp_w[1].start()
        xb = x_ref[i * RB:(i + 1) * RB, :]
        ks = jnp.concatenate(
            [jnp.dot(xb[t * 128:(t + 1) * 128], wk_ref[...], preferred_element_type=F32)
             for t in range(RB // 128)], axis=0)
        ka = jnp.max(jnp.abs(ks).reshape(RB // 8, 8, D), axis=0)
        k2 = jnp.sum((ks * ks).reshape(RB // 8, 8, D), axis=0)
        kamax = ka if kamax is None else jnp.maximum(kamax, ka)
        ksq = k2 if ksq is None else ksq + k2
        for t in range(NT5):
            kf_ref[t, i * RB:(i + 1) * RB, :] = ks[:, 128 * t:128 * (t + 1)]
        if i == 2:
            wqvt_ref[0:D, :] = wq_ref[...].astype(F32).T.astype(BF16)
    kmax0 = jnp.max(kamax, axis=0, keepdims=True)
    kmax = jnp.maximum(kmax0, 1e-30)
    kinv = 1.0 / kmax
    kms = jnp.sum(ksq, axis=0, keepdims=True) * (1.0 / S) * kinv * kinv
    kok = jnp.min(jnp.where((kms >= 0.16 ** 2) | (kmax0 == 0.0), 1.0, 0.0), axis=1, keepdims=True)
    kcol = jnp.concatenate(
        [jnp.broadcast_to(kmax[:, 128 * t:128 * (t + 1)] * QSCALE, (128, 128)).T for t in range(NT5)], axis=0)
    yscale8 = jnp.broadcast_to(kinv * YMAX, (8, D))

    z0 = lax.bitcast_convert_type(kf_ref[0, 0:8, :], I32) | 1

    QR = 32
    qlane = lax.broadcasted_iota(I32, (QR // 4, 128), 1)

    def kq_job(tie, rb):
        rows = slice(rb * QR, (rb + 1) * QR)
        tiles = [kf_ref[t, rows, :] for t in range(NT5)]
        ys = tied(yscale8, tie, z0)
        y = jnp.concatenate(tiles, axis=1) * jnp.concatenate([ys] * (QR // 8), axis=0)
        b = iround(y)
        b1 = iround(y * (1.0 / 3.0))
        b3 = b - b1 - b1
        rb16 = iround((y - b.astype(F32)) * 16.0)
        y16 = iround(y * (1.0 / 16.0))
        p1, p3, p4, p5 = pk8(b1), pk8(b3), pk8(rb16), pk8(y16)
        for j in range(NSLAB):
            sh = 8 * j
            for arr, ms in ((p1, (0, 1)), (p3, (2,)), (p4, (3,)), (p5, (4,))):
                if j == 0:
                    sl = arr[:, 0:128]
                elif j < NSLAB - 1:
                    sl = jnp.where(qlane >= 128 - sh, arr[:, 128 * (j - 1):128 * j], arr[:, 128 * j:128 * (j + 1)])
                else:
                    sl = arr[:, 128 * (j - 1):128 * j]
                for m in ms:
                    tot = (sh + HP * m) % 128
                    r8_ref[j, m, rb * (QR // 4):(rb + 1) * (QR // 4), :] = pltpu.roll(sl, tot, 1) if tot else sl

    AR = 64
    alane = lax.broadcasted_iota(I32, (AR, 128), 1)
    QW = 256
    r24 = lax.broadcasted_iota(I32, (HP, QW), 0)

    def prep_jobs(h0, W, zt):
        jobs = []
        for par in range(2):
            h = h0 + par
            j = h // HPS
            lo = (h % HPS) * DH
            off = 4 * par
            for part in range(8):
                def kjob(tie, part=part, par=par, j=j, lo=lo, off=off):
                    rel = (alane - lo) & 127
                    rows = slice(part * AR, (part + 1) * AR)
                    v = tied(jnp.full((AR, 128), 0x7F7F7F7F, I32), tie, zt)
                    for m in range(NLIMB):
                        v = jnp.where((rel >= HP * m) & (rel < HP * m + DH), r8_ref[j, m, rows, :], v)
                    W['k8'][pl.ds(par * (S // 4) + part * AR, AR), :] = pltpu.roll(v, (128 + off - lo) % 128, 1)
                jobs.append((1, "k", kjob))

                def qjob(tie, qi=part // 2, ls=slice((part % 2) * QW, (part % 2 + 1) * QW), par=par, h=h, off=off):
                    w0 = h * DH - off
                    if not isinstance(w0, int):
                        w0 = pl.multiple_of(w0, 8)
                    valid = (r24 >= off) & (r24 < off + DH)
                    w = tied(qt_ref[qi, pl.ds(w0, HP), ls], tie, zt)
                    w = jnp.where(valid, w, 0.0)
                    amax = jnp.maximum(jnp.max(jnp.abs(w), axis=0, keepdims=True), 1e-30)
                    xq = w * (127.0 / amax)
                    nrm = jnp.sqrt(jnp.sum(xq * xq, axis=0, keepdims=True))
                    cs = iround(nrm * (-0.9 * YMAX / (127.0 * NSH)))
                    a1 = iround(xq)
                    a16 = iround(xq * (1.0 / 16.0))
                    ra16 = iround((xq - a1.astype(F32)) * 16.0)
                    a1, a16, ra16 = (jnp.where(valid, t_, cs) for t_ in (a1, a16, ra16))
                    op = jnp.concatenate([a1, a1, a1, a16, ra16, jnp.broadcast_to(cs, (8, QW))], axis=0)
                    st = par * NQ + qi
                    W['qz'][pl.ds(st * 32, 32), ls] = pk8(op)
                    W['fq'][pl.ds(st * 8, 8), ls] = jnp.broadcast_to(amax * (1.0 / (127.0 * YMAX)), (8, QW))
                jobs.append((2, "q", qjob))
        return jobs

    def views(z):
        return dict(k8=zview(k8_ref, z), qz=zview(qz_ref, z), fq=zview(fq_ref, z), p=[zview(r, z) for r in pbuf])

    wjobs = []
    for r in range(D // 16):
        def w1job(tie, r=r):
            w1p_ref[8 * r:8 * r + 8, :] = tied(pk(w1_ref[16 * r:16 * r + 16, :]), tie, z0)
        wjobs.append(w1job)
    for r in range(DFF // 32):
        def w2job(tie, r=r):
            w2p_ref[16 * r:16 * r + 16, :] = tied(pk(w2_ref[32 * r:32 * r + 32, :]), tie, z0)
        wjobs.append(w2job)
    kqjobs = [(lambda tie, rb=rb: kq_job(tie, rb)) for rb in range(S // QR)]
    NKQ = len(kqjobs)
    kqsplit = [0, 10, 20, 28, 36, 46, 56, 64]

    qamax = None
    for i in range(NB):
        xb = x_ref[i * RB:(i + 1) * RB, :]
        if i == 2:
            cp_wv.wait()
            cp_w[0].wait()
            cp_w[1].wait()
            cp_w[2].start()
            wqvt_ref[D:2 * D, :] = wv_ref[...].astype(F32).T.astype(BF16)
        q = lax.dot_general(wqvt_ref[0:D, :], xb, NT, preferred_element_type=F32)
        q = q * jnp.concatenate([kcol] * (RB // 128), axis=1)
        qa = jnp.max(jnp.abs(q).reshape(D // 8, 8, RB), axis=0)
        qamax = qa if qamax is None else jnp.maximum(qamax, qa)
        qt_ref[i] = q
        spread(kqjobs[kqsplit[i]:kqsplit[i + 1]], q)
        if i >= 2:
            spread(wjobs[(i - 2) * 44:(i - 1) * 44], q)
    fmax = jnp.max(jnp.max(qamax, axis=0, keepdims=True), axis=1, keepdims=True) * (1.0 / (127.0 * YMAX))
    limb_ok = jnp.maximum(kok, jnp.where(fmax * 12.0 <= 2.0 ** -9, 1.0, 0.0))

    gw16 = jnp.broadcast_to(gw_ref[...].astype(F32).reshape(1, D), (16, D)).astype(BF16)
    for i in range(NB):
        cs = slice(i * RB, (i + 1) * RB)
        xb = x_ref[cs, :]
        v = lax.dot_general(jnp.concatenate([wqvt_ref[D:, :], gw16], axis=0), xb, NT, preferred_element_type=F32)
        for p in range(H // 2):
            g = v[40 * p:40 * p + 40]
            mid = g[16:24]
            vt_ref[48 * p:48 * p + 16, cs] = g[0:16]
            vt_ref[48 * p + 16:48 * p + 24, cs] = jnp.where(r8 < 4, mid, jnp.where(r8 == 4, 1.0, 0.0))
            vt_ref[48 * p + 24:48 * p + 32, cs] = jnp.where(r8 >= 4, mid, jnp.where(r8 == 0, 1.0, 0.0))
            vt_ref[48 * p + 32:48 * p + 48, cs] = g[24:40]
        grow = jax.nn.sigmoid(v[D:D + 8])
        for t in range(RB // 128):
            gb = jnp.concatenate([grow[:, 128 * t:128 * (t + 1)]] * 16, axis=0)
            g_ref[i * RB + 128 * t:i * RB + 128 * (t + 1), :] = gb.T
        if i < 3:
            spread(kqjobs[kqsplit[4 + i]:kqsplit[5 + i]], v[0:D])
        if i == 2:
            for _, _, f_ in prep_jobs(0, views(0), z0):
                f_(None)

    lastacc = [None]

    def stage(cur, prev, W, R, ztrue, do_a=True):
        hp, qp, orow = prev
        vrow = pl.multiple_of(hp * HP, 8)
        acc = None
        wbase = (cur % 2) * NPER * HK
        rbase = ((cur + 1) % 2) * NPER * HK
        par = cur // NQ
        for c in range(NKC):
            vt = vt_ref[pl.ds(vrow, HP), c * KC:(c + 1) * KC]
            pw = R['p'][c % NP][pl.ds(rbase + (c // NP) * HK, HK), :]
            d = jnp.dot(vt, upk(pw), preferred_element_type=F32)
            if acc is None:
                acc = d if lastacc[0] is None else jnp.where(ztrue, d, lastacc[0])
            else:
                acc = acc + d
            if not do_a:
                continue
            s = jnp.dot(up8(R['k8'][pl.ds(par * (S // 4) + c * (KC // 4), KC // 4), :]),
                        up8(R['qz'][pl.ds(cur * 32, 32), :]), preferred_element_type=I32)
            f = R['fq'][pl.ds(cur * 8, 8), :]
            t = s.astype(F32) * jnp.concatenate([f] * (KC // 8), axis=0)
            W['p'][c % NP][pl.ds(wbase + (c // NP) * HK, HK), :] = pk(jnp.exp2(t).astype(BF16))
        ot_ref[pl.ds(pl.multiple_of(orow, 8), HP), qp * TQ:(qp + 1) * TQ] = acc
        lastacc[0] = acc

    def body(u, carry):
        z = lax.shift_right_logical(u, 8)
        z2 = lax.shift_right_logical(u, 9)
        W = views(z)
        R = views(z2)
        ztrue = z2 == 0
        lastacc[0] = None
        for i in range(U):
            if i == 0:
                hp = jnp.maximum(2 * u - 1, 0)
                prev = (hp, NQ - 1, jnp.where(u == 0, H * HP, hp * HP))
            else:
                hp = 2 * u + (i - 1) // NQ
                prev = (hp, (i - 1) % NQ, hp * HP)
            stage(i, prev, W, R, ztrue)

        rs = pl.ds(pl.multiple_of(u * FR, FR), FR)
        xb = x_ref[rs, :]
        jobs = [f_ for _, _, f_ in prep_jobs(jnp.minimum(2 * u + 2, H - 2), W, z)]
        hs = []
        for n in range(3):
            hf = jnp.maximum(jnp.dot(xb, upk(w1p_ref[:, 512 * n:512 * (n + 1)]), preferred_element_type=F32), 0.0)
            spread(jobs[6 * n:6 * n + 6], hf)
            hs.append(hf.astype(BF16))
        g1 = 1.0 - g_ref[rs, :]
        nj = 18
        for n in range(5):
            bn = None
            for kk in range(3):
                pd = jnp.dot(hs[kk], upk(w2p_ref[256 * kk:256 * (kk + 1), 128 * n:128 * (n + 1)]),
                             preferred_element_type=F32)
                bn = pd if bn is None else bn + pd
                if nj < len(jobs):
                    jobs[nj](pd[0:8])
                    nj += 1
            bm_ref[rs, 128 * n:128 * (n + 1)] = g1 * bn
        assert nj == len(jobs)
        return carry
    lax.fori_loop(0, NIT, body, 0)
    lastacc[0] = None
    stage(0, (H - 1, NQ - 1, (H - 1) * HP), None, views(0), None, do_a=False)

    cp_w[2].wait()

    def rows_of(i):
        return pl.ds(i * FB, FB) if isinstance(i, int) else pl.ds(pl.multiple_of(i * FB, FB), FB)

    def out_cp(i):
        return pltpu.make_async_copy(out_ref.at[rows_of(i)], out_hbm.at[rows_of(i)], sem_out.at[i])

    r8f = lax.broadcasted_iota(I32, (8, FB), 0)

    def fin(i, check):
        rs = rows_of(i)
        parts = []
        lmin = amax = None
        for p in range(H // 2):
            e = ot_ref[48 * p:48 * p + 24, rs]
            o = ot_ref[48 * p + 24:48 * p + 48, rs]
            if check:
                l = jnp.where(r8f < 4, o[0:8], e[16:24])
                lmin = l if lmin is None else jnp.minimum(lmin, l)
                for t_ in (e, o):
                    am = jnp.max(jnp.abs(t_).reshape(3, 8, FB), axis=0)
                    amax = am if amax is None else jnp.maximum(amax, am)
            e = e * (1.0 / e[DH:DH + 1])
            o = o * (1.0 / o[0:1])
            parts += [e[0:16], jnp.where(r8f < 4, e[16:24], o[0:8]), o[8:24]]
        ot = jnp.concatenate(parts, axis=0).T.astype(BF16)
        a = jnp.dot(ot, wo_ref[...], preferred_element_type=F32)
        g = jnp.concatenate([g_ref[rs, :]] * (D // 128), axis=1)
        out_ref[rs, :] = (g * a + bm_ref[rs, :]).astype(out_ref.dtype)
        out_cp(i).start()
        if check:
            ok = ((lmin >= 2.0 ** -60) | ((r8f != 0) & (r8f != 4))) & (amax <= 2.0 ** 120)
            return jnp.where(ok, 0.0, 1.0)

    bad = None
    for i in range(NFB):
        bi = fin(i, True)
        bad = bi if bad is None else jnp.maximum(bad, bi)
    nbad = jnp.max(jnp.max(bad, axis=1, keepdims=True), axis=0, keepdims=True) + (1.0 - limb_ok)
    nbad = nbad[0, 0]
    for i in range(NFB):
        out_cp(i).wait()

    @pl.when(nbad > 0.0)
    def _():
        def norm(i, c):
            rs = pl.ds(pl.multiple_of(i * 256, 256), 256)
            for t in range(NT5):
                kf_ref[t, rs, :] = kf_ref[t, rs, :] * kinv[:, 128 * t:128 * (t + 1)]
            return c
        lax.fori_loop(0, S // 256, norm, 0)
        qrow = lax.broadcasted_iota(I32, (128, TQ), 0)

        def fb(t, c):
            h = t // NQ
            qi = t % NQ
            t0 = jnp.minimum((h * DH) // 128, NT5 - 2)
            s = None
            for tt in range(2):
                r0 = pl.multiple_of((t0 + tt) * 128, 128)
                fr = qrow + r0
                qz = jnp.where((fr >= h * DH) & (fr < h * DH + DH), qt_ref[qi, pl.ds(r0, 128), :], 0.0).astype(BF16)
                sp = jnp.dot(kf_ref[t0 + tt].astype(BF16), qz, preferred_element_type=F32)
                s = sp if s is None else s + sp
            m = jnp.max(s, axis=0, keepdims=True)
            p = jnp.exp2(s - m).astype(BF16)
            vrow = pl.multiple_of(h * HP, 8)
            acc = jnp.dot(vt_ref[pl.ds(vrow, HP), :], p, preferred_element_type=F32)
            ot_ref[pl.ds(vrow, HP), pl.ds(pl.multiple_of(qi * TQ, TQ), TQ)] = acc
            return c
        lax.fori_loop(0, NSTEP, fb, 0)

        def fin2(i, c):
            fin(i, False)
            out_cp(i).wait()
            return c
        lax.fori_loop(0, NFB, fin2, 0)


_SCRATCH = [
    pltpu.VMEM((S, D), BF16),
    pltpu.VMEM((D, D), BF16),
    pltpu.VMEM((D, D), BF16),
    pltpu.VMEM((D, D), BF16),
    pltpu.VMEM((D, D), BF16),
    pltpu.VMEM((D, DFF), BF16),
    pltpu.VMEM((DFF, D), BF16),
    pltpu.VMEM((S, D), BF16),
    pltpu.VMEM((2 * D, D), BF16),
    pltpu.VMEM((D // 2, DFF), F32),
    pltpu.VMEM((DFF // 2, D), F32),
    pltpu.VMEM((NT5, S, 128), F32),
    pltpu.VMEM((NSLAB, NLIMB, S // 4, 128), I32),
    pltpu.VMEM((NQ, D, TQ), F32),
    pltpu.VMEM((H * HP, S), F32),
    pltpu.VMEM((H * HP + HP, S), F32),
    pltpu.VMEM((S, D), F32),
    pltpu.VMEM((S, 128), F32),
    pltpu.VMEM((2 * S // 4, 128), I32),
    pltpu.VMEM((U * 32, TQ), I32),
    pltpu.VMEM((U * 8, TQ), F32),
] + [pltpu.VMEM((2 * NPER * HK, TQ), F32)] * NP + [
    pltpu.SemaphoreType.DMA((6,)),
    pltpu.SemaphoreType.DMA((NB,)),
    pltpu.SemaphoreType.DMA((NFB,)),
]


@jax.jit
def pallas_gated_mix__softmax_full_mha__dense_activation_relu__prompt_kernel(
    A_x: jax.Array,
    A_wqkv: jax.Array,
    A_wo: jax.Array,
    B_x: jax.Array,
    B_w1: jax.Array,
    B_w2: jax.Array,
    gate_w: jax.Array,
):
    anyspec = pl.BlockSpec(memory_space=pl.ANY)
    out = pl.pallas_call(
        _kernel,
        out_shape=jax.ShapeDtypeStruct((S, D), BF16),
        in_specs=[anyspec] * 5 + [pl.BlockSpec(memory_space=pltpu.VMEM)],
        out_specs=anyspec,
        scratch_shapes=_SCRATCH,
        compiler_params=pltpu.CompilerParams(vmem_limit_bytes=100 * 1024 * 1024),
    )(A_x.reshape(S, D), A_wqkv, A_wo, B_w1, B_w2, gate_w)
    return out.reshape(1, S, D)
```

```python
import math

import jax
import jax.numpy as jnp
from jax import lax
import jax.experimental.pallas as pl
import jax.experimental.pallas.tpu as pltpu

S, D, H, DH, DFF = 2048, 640, 32, 20, 1536
HP = 24
HPS = 6
NSLAB = 6
SLABW = HPS * DH
NT5 = D // 128
F32 = jnp.float32
BF16 = jnp.bfloat16
I32 = jnp.int32
I8 = jnp.int8

TQ = 512
KC = 512
NP = 2
FB = 128
WB = 2
RB = TQ
NB = S // RB
NQ = S // TQ
NFB = S // FB
NSTEP = H * NQ
NKC = S // KC
NPER = NKC // NP
HK = KC // 2
U = 2 * NQ
NIT = NSTEP // U
FR = S // NIT
QSCALE = (DH ** -0.5) * math.log2(math.e)
YMAX = 378.0
NLIMB = 5
NSH = 128 - NLIMB * DH

NT = (((1,), (1,)), ((), ()))


def pk(x):
    return pltpu.bitcast(x, F32)


def upk(x):
    return pltpu.bitcast(x, BF16)


def pk8(x):
    return pltpu.bitcast(x.astype(I8), I32)


def up8(x):
    return pltpu.bitcast(x, I8)


def iround(x):
    return jnp.round(x).astype(I32)


def zview(ref, z):
    if isinstance(z, int):
        return ref
    return ref.at[pl.ds(pl.multiple_of(z * 8, 8), ref.shape[0])]


def tied(v, tie, zt):
    if tie is None:
        return v
    if tie.dtype != v.dtype:
        tie = lax.bitcast_convert_type(tie, v.dtype)
    t = jnp.concatenate([tie] * (v.shape[1] // 128), axis=1)
    t = jnp.concatenate([t] * (v.shape[0] // 8), axis=0)
    if zt.ndim:
        m = jnp.concatenate([zt] * (v.shape[1] // 128), axis=1)
        m = jnp.concatenate([m] * (v.shape[0] // 8), axis=0)
        return jnp.where(m != 0, v, t)
    return jnp.where(zt == 0, v, t)


def spread(fns, val):
    nr = val.shape[0] // 8
    nv = nr * (val.shape[1] // 128)
    for n_, fn in enumerate(fns):
        col, row = divmod((n_ * nv) // len(fns), nr)
        fn(val[8 * row:8 * row + 8, 128 * col:128 * (col + 1)])


def _kernel(x_hbm, wqkv_hbm, wo_hbm, w1_hbm, w2_hbm, gw_hbm, out_hbm,
            x_ref, wq_ref, wk_ref, wv_ref, wo_ref, w1_ref, w2_ref, out_ref,
            wqvt_ref, w1p_ref, w2p_ref, kf_ref, r8_ref, qt_ref, vt_ref, ot_ref, bm_ref, g_ref,
            k8_ref, qz_ref, fq_ref, *rest):
    pbuf = rest[:NP]
    gw_ref, sem_in, sem_x, sem_out = rest[NP:]

    cp_wk = pltpu.make_async_copy(wqkv_hbm.at[:, D:2 * D], wk_ref, sem_in.at[0])
    cp_wq = pltpu.make_async_copy(wqkv_hbm.at[:, 0:D], wq_ref, sem_in.at[1])
    cp_wv = pltpu.make_async_copy(wqkv_hbm.at[:, 2 * D:3 * D], wv_ref, sem_in.at[2])
    cp_x = [pltpu.make_async_copy(x_hbm.at[i * RB:(i + 1) * RB], x_ref.at[i * RB:(i + 1) * RB], sem_x.at[i])
            for i in range(NB)]
    cp_w = [pltpu.make_async_copy(a, b, sem_in.at[3 + n])
            for n, (a, b) in enumerate(((w1_hbm, w1_ref), (w2_hbm, w2_ref), (wo_hbm, wo_ref)))]
    cp_gw = pltpu.make_async_copy(gw_hbm, gw_ref, sem_in.at[6])
    cp_wk.start()
    cp_x[0].start()
    for pb in pbuf:
        pb[NPER * HK:2 * NPER * HK, :] = jnp.zeros((NPER * HK, TQ), F32)
    cp_wk.wait()
    cp_x[1].start()
    r8 = lax.broadcasted_iota(I32, (8, RB), 0)

    kamax = ksq = None
    for i in range(NB):
        if i == 0:
            cp_x[0].wait()
            cp_x[2].start()
            cp_x[3].start()
        if i == 1:
            cp_wq.start()
            cp_x[1].wait()
        if i == 2:
            cp_x[2].wait()
            cp_x[3].wait()
            cp_wv.start()
            cp_gw.start()
            cp_w[0].start()
            cp_w[1].start()
            cp_wq.wait()
        xb = x_ref[i * RB:(i + 1) * RB, :]
        ks = jnp.concatenate(
            [jnp.dot(xb[t * 128:(t + 1) * 128], wk_ref[...], preferred_element_type=F32)
             for t in range(RB // 128)], axis=0)
        ka = jnp.max(jnp.abs(ks).reshape(RB // 8, 8, D), axis=0)
        k2 = jnp.sum((ks * ks).reshape(RB // 8, 8, D), axis=0)
        kamax = ka if kamax is None else jnp.maximum(kamax, ka)
        ksq = k2 if ksq is None else ksq + k2
        for t in range(NT5):
            kf_ref[t, i * RB:(i + 1) * RB, :] = ks[:, 128 * t:128 * (t + 1)]
        if i == 2:
            wqvt_ref[0:D, :] = wq_ref[...].astype(F32).T.astype(BF16)
    kmax0 = jnp.max(kamax, axis=0, keepdims=True)
    kmax = jnp.maximum(kmax0, 1e-30)
    kinv = 1.0 / kmax
    kms = jnp.sum(ksq, axis=0, keepdims=True) * (1.0 / S) * kinv * kinv
    kok = jnp.min(jnp.where(((kms >= 0.14 ** 2) & (kms <= 1.01)) | (kmax0 == 0.0), 1.0, 0.0),
                  axis=1, keepdims=True)
    kcol = jnp.concatenate(
        [jnp.broadcast_to(kmax[:, 128 * t:128 * (t + 1)] * QSCALE, (128, 128)).T for t in range(NT5)], axis=0)
    yscale8 = jnp.broadcast_to(kinv * YMAX, (8, D))

    z0 = lax.bitcast_convert_type(kf_ref[0, 0:8, :], I32) | 1

    QR = 32
    qlane = lax.broadcasted_iota(I32, (QR // 4, 128), 1)

    def kq_job(tie, rb):
        rows = slice(rb * QR, (rb + 1) * QR)
        tiles = [kf_ref[t, rows, :] for t in range(NT5)]
        ys = tied(yscale8, tie, z0)
        y = jnp.concatenate(tiles, axis=1) * jnp.concatenate([ys] * (QR // 8), axis=0)
        b = iround(y)
        b1 = iround(y * (1.0 / 3.0))
        b3 = b - b1 - b1
        rb16 = iround((y - b.astype(F32)) * 16.0)
        y16 = iround(y * (1.0 / 16.0))
        p1, p3, p4, p5 = pk8(b1), pk8(b3), pk8(rb16), pk8(y16)
        for j in range(NSLAB):
            sh = 8 * j
            for arr, ms in ((p1, (0, 1)), (p3, (2,)), (p4, (3,)), (p5, (4,))):
                if j == 0:
                    sl = arr[:, 0:128]
                elif j < NSLAB - 1:
                    sl = jnp.where(qlane >= 128 - sh, arr[:, 128 * (j - 1):128 * j], arr[:, 128 * j:128 * (j + 1)])
                else:
                    sl = arr[:, 128 * (j - 1):128 * j]
                for m in ms:
                    tot = (sh + HP * m) % 128
                    r8_ref[j, m, rb * (QR // 4):(rb + 1) * (QR // 4), :] = pltpu.roll(sl, tot, 1) if tot else sl

    AR = 64
    alane = lax.broadcasted_iota(I32, (AR, 128), 1)
    QW = 256
    r24 = lax.broadcasted_iota(I32, (HP, QW), 0)

    def prep_jobs(h0, W, zt):
        jobs = []
        for par in range(2):
            h = h0 + par
            j = h // HPS
            lo = (h % HPS) * DH
            off = 4 * par
            for part in range(8):
                def kjob(tie, part=part, par=par, j=j, lo=lo, off=off):
                    rel = (alane - lo) & 127
                    rows = slice(part * AR, (part + 1) * AR)
                    v = tied(jnp.full((AR, 128), 0x7F7F7F7F, I32), tie, zt)
                    for m in range(NLIMB):
                        v = jnp.where((rel >= HP * m) & (rel < HP * m + DH), r8_ref[j, m, rows, :], v)
                    W['k8'][pl.ds(par * (S // 4) + part * AR, AR), :] = pltpu.roll(v, (128 + off - lo) % 128, 1)
                jobs.append((1, "k", kjob))

                def qjob(tie, qi=part // 2, ls=slice((part % 2) * QW, (part % 2 + 1) * QW), par=par, h=h, off=off):
                    w0 = h * DH - off
                    if not isinstance(w0, int):
                        w0 = pl.multiple_of(w0, 8)
                    valid = (r24 >= off) & (r24 < off + DH)
                    w = tied(qt_ref[qi, pl.ds(w0, HP), ls], tie, zt)
                    w = jnp.where(valid, w, 0.0)
                    amax = jnp.maximum(jnp.max(jnp.abs(w), axis=0, keepdims=True), 1e-30)
                    xq = w * (127.0 / amax)
                    nrm = jnp.sqrt(jnp.sum(xq * xq, axis=0, keepdims=True))
                    cs = iround(nrm * (-0.9 * YMAX / (127.0 * NSH)))
                    a1 = iround(xq)
                    a16 = iround(xq * (1.0 / 16.0))
                    ra16 = iround((xq - a1.astype(F32)) * 16.0)
                    a1, a16, ra16 = (jnp.where(valid, t_, cs) for t_ in (a1, a16, ra16))
                    op = jnp.concatenate([a1, a1, a1, a16, ra16, jnp.broadcast_to(cs, (8, QW))], axis=0)
                    st = par * NQ + qi
                    W['qz'][pl.ds(st * 32, 32), ls] = pk8(op)
                    W['fq'][pl.ds(st * 8, 8), ls] = jnp.broadcast_to(amax * (1.0 / (127.0 * YMAX)), (8, QW))
                jobs.append((2, "q", qjob))
        return jobs

    def views(z):
        return dict(k8=zview(k8_ref, z), qz=zview(qz_ref, z), fq=zview(fq_ref, z), p=[zview(r, z) for r in pbuf])

    wjobs = []
    for r in range(D // 16):
        def w1job(tie, r=r):
            w1p_ref[8 * r:8 * r + 8, :] = tied(pk(w1_ref[16 * r:16 * r + 16, :]), tie, z0)
        wjobs.append(w1job)
    for r in range(DFF // 32):
        def w2job(tie, r=r):
            w2p_ref[16 * r:16 * r + 16, :] = tied(pk(w2_ref[32 * r:32 * r + 32, :]), tie, z0)
        wjobs.append(w2job)
    kqjobs = [(lambda tie, rb=rb: kq_job(tie, rb)) for rb in range(S // QR)]
    kqsplit = [0, 12, 22, 25, 28, 41, 54, 64]

    qamax = None
    for i in range(NB):
        xb = x_ref[i * RB:(i + 1) * RB, :]
        if i == WB:
            cp_wv.wait()
            cp_gw.wait()
            cp_w[0].wait()
            cp_w[2].start()
            cp_w[1].wait()
            wqvt_ref[D:2 * D, :] = wv_ref[...].astype(F32).T.astype(BF16)
        q = lax.dot_general(wqvt_ref[0:D, :], xb, NT, preferred_element_type=F32)
        q = q * jnp.concatenate([kcol] * (RB // 128), axis=1)
        qa = jnp.max(jnp.abs(q).reshape(D // 8, 8, RB), axis=0)
        qamax = qa if qamax is None else jnp.maximum(qamax, qa)
        qt_ref[i] = q
        spread(kqjobs[kqsplit[i]:kqsplit[i + 1]], q)
        if i >= WB:
            spread(wjobs[(i - WB) * 88 // (NB - WB):(i - WB + 1) * 88 // (NB - WB)], q)
    fmax = jnp.max(jnp.max(qamax, axis=0, keepdims=True), axis=1, keepdims=True) * (1.0 / (127.0 * YMAX))
    limb_ok = jnp.maximum(kok, jnp.where(fmax * 12.0 <= 2.0 ** -9, 1.0, 0.0))

    gw16 = jnp.broadcast_to(gw_ref[...].astype(F32).reshape(1, D), (16, D)).astype(BF16)
    for i in range(NB):
        cs = slice(i * RB, (i + 1) * RB)
        xb = x_ref[cs, :]
        v = lax.dot_general(jnp.concatenate([wqvt_ref[D:, :], gw16], axis=0), xb, NT, preferred_element_type=F32)
        for p in range(H // 2):
            g = v[40 * p:40 * p + 40]
            mid = g[16:24]
            vt_ref[48 * p:48 * p + 16, cs] = g[0:16]
            vt_ref[48 * p + 16:48 * p + 24, cs] = jnp.where(r8 < 4, mid, jnp.where(r8 == 4, 1.0, 0.0))
            vt_ref[48 * p + 24:48 * p + 32, cs] = jnp.where(r8 >= 4, mid, jnp.where(r8 == 0, 1.0, 0.0))
            vt_ref[48 * p + 32:48 * p + 48, cs] = g[24:40]
        grow = jax.nn.sigmoid(v[D:D + 8])
        for t in range(RB // 128):
            gb = jnp.concatenate([grow[:, 128 * t:128 * (t + 1)]] * 16, axis=0)
            g_ref[i * RB + 128 * t:i * RB + 128 * (t + 1), :] = gb.T
        if i < 3:
            spread(kqjobs[kqsplit[4 + i]:kqsplit[5 + i]], v[0:D])
        if i == 2:
            for _, _, f_ in prep_jobs(0, views(0), z0):
                f_(None)

    lastacc = [None]

    def stage(cur, prev, W, R, ztrue, do_a=True):
        hp, qp, orow = prev
        vrow = pl.multiple_of(hp * HP, 8)
        acc = None
        wbase = (cur % 2) * NPER * HK
        rbase = ((cur + 1) % 2) * NPER * HK
        par = cur // NQ
        for c in range(NKC):
            vt = vt_ref[pl.ds(vrow, HP), c * KC:(c + 1) * KC]
            pw = R['p'][c % NP][pl.ds(rbase + (c // NP) * HK, HK), :]
            d = jnp.dot(vt, upk(pw), preferred_element_type=F32)
            if acc is None:
                acc = d if lastacc[0] is None else jnp.where(ztrue, d, lastacc[0])
            else:
                acc = acc + d
            if not do_a:
                continue
            s = jnp.dot(up8(R['k8'][pl.ds(par * (S // 4) + c * (KC // 4), KC // 4), :]),
                        up8(R['qz'][pl.ds(cur * 32, 32), :]), preferred_element_type=I32)
            f = R['fq'][pl.ds(cur * 8, 8), :]
            t = s.astype(F32) * jnp.concatenate([f] * (KC // 8), axis=0)
            W['p'][c % NP][pl.ds(wbase + (c // NP) * HK, HK), :] = pk(jnp.exp2(t).astype(BF16))
        ot_ref[pl.ds(pl.multiple_of(orow, 8), HP), qp * TQ:(qp + 1) * TQ] = acc
        lastacc[0] = acc

    def body(u, carry):
        z = lax.shift_right_logical(u, 8)
        z2 = lax.shift_right_logical(u, 9)
        W = views(z)
        R = views(z2)
        ztrue = z2 == 0
        lastacc[0] = None
        for i in range(U):
            if i == 0:
                hp = jnp.maximum(2 * u - 1, 0)
                prev = (hp, NQ - 1, jnp.where(u == 0, H * HP, hp * HP))
            else:
                hp = 2 * u + (i - 1) // NQ
                prev = (hp, (i - 1) % NQ, hp * HP)
            stage(i, prev, W, R, ztrue)

        rs = pl.ds(pl.multiple_of(u * FR, FR), FR)
        xb = x_ref[rs, :]
        jobs = [f_ for _, _, f_ in prep_jobs(jnp.minimum(2 * u + 2, H - 2), W, z)]
        hs = []
        for n in range(3):
            hf = jnp.maximum(jnp.dot(xb, upk(w1p_ref[:, 512 * n:512 * (n + 1)]), preferred_element_type=F32), 0.0)
            spread(jobs[6 * n:6 * n + 6], hf)
            hs.append(hf.astype(BF16))
        g1 = 1.0 - g_ref[rs, :]
        nj = 18
        for n in range(5):
            bn = None
            for kk in range(3):
                pd = jnp.dot(hs[kk], upk(w2p_ref[256 * kk:256 * (kk + 1), 128 * n:128 * (n + 1)]),
                             preferred_element_type=F32)
                bn = pd if bn is None else bn + pd
                if nj < len(jobs):
                    jobs[nj](pd[0:8])
                    nj += 1
            bm_ref[rs, 128 * n:128 * (n + 1)] = g1 * bn
        assert nj == len(jobs)
        return carry
    lax.fori_loop(0, NIT, body, 0)
    lastacc[0] = None
    stage(0, (H - 1, NQ - 1, (H - 1) * HP), None, views(0), None, do_a=False)

    cp_w[2].wait()

    def rows_of(i):
        return pl.ds(i * FB, FB) if isinstance(i, int) else pl.ds(pl.multiple_of(i * FB, FB), FB)

    def out_cp(i):
        return pltpu.make_async_copy(out_ref.at[rows_of(i)], out_hbm.at[rows_of(i)], sem_out.at[i])

    r8f = lax.broadcasted_iota(I32, (8, FB), 0)

    def fin(i, check):
        rs = rows_of(i)
        parts = []
        lmin = amax = None
        for p in range(H // 2):
            e = ot_ref[48 * p:48 * p + 24, rs]
            o = ot_ref[48 * p + 24:48 * p + 48, rs]
            if check:
                l = jnp.where(r8f < 4, o[0:8], e[16:24])
                lmin = l if lmin is None else jnp.minimum(lmin, l)
                for t_ in (e, o):
                    am = jnp.max(jnp.abs(t_).reshape(3, 8, FB), axis=0)
                    amax = am if amax is None else jnp.maximum(amax, am)
            e = e * (1.0 / e[DH:DH + 1])
            o = o * (1.0 / o[0:1])
            parts += [e[0:16], jnp.where(r8f < 4, e[16:24], o[0:8]), o[8:24]]
        ot = jnp.concatenate(parts, axis=0).T.astype(BF16)
        a = jnp.dot(ot, wo_ref[...], preferred_element_type=F32)
        g = jnp.concatenate([g_ref[rs, :]] * (D // 128), axis=1)
        out_ref[rs, :] = (g * a + bm_ref[rs, :]).astype(out_ref.dtype)
        out_cp(i).start()
        if check:
            ok = ((lmin >= 2.0 ** -60) | ((r8f != 0) & (r8f != 4))) & (amax <= 2.0 ** 120)
            return jnp.where(ok, 0.0, 1.0)

    bad = None
    for i in range(NFB):
        bi = fin(i, True)
        bad = bi if bad is None else jnp.maximum(bad, bi)
    nbad = jnp.max(jnp.max(bad, axis=1, keepdims=True), axis=0, keepdims=True) + (1.0 - limb_ok)
    nbad = nbad[0, 0]
    for i in range(NFB):
        out_cp(i).wait()

    @pl.when(nbad > 0.0)
    def _():
        def norm(i, c):
            rs = pl.ds(pl.multiple_of(i * 256, 256), 256)
            for t in range(NT5):
                kf_ref[t, rs, :] = kf_ref[t, rs, :] * kinv[:, 128 * t:128 * (t + 1)]
            return c
        lax.fori_loop(0, S // 256, norm, 0)
        qrow = lax.broadcasted_iota(I32, (128, TQ), 0)

        def fb(t, c):
            h = t // NQ
            qi = t % NQ
            t0 = jnp.minimum((h * DH) // 128, NT5 - 2)
            s = None
            for tt in range(2):
                r0 = pl.multiple_of((t0 + tt) * 128, 128)
                fr = qrow + r0
                qz = jnp.where((fr >= h * DH) & (fr < h * DH + DH), qt_ref[qi, pl.ds(r0, 128), :], 0.0).astype(BF16)
                sp = jnp.dot(kf_ref[t0 + tt].astype(BF16), qz, preferred_element_type=F32)
                s = sp if s is None else s + sp
            m = jnp.max(s, axis=0, keepdims=True)
            p = jnp.exp2(s - m).astype(BF16)
            vrow = pl.multiple_of(h * HP, 8)
            acc = jnp.dot(vt_ref[pl.ds(vrow, HP), :], p, preferred_element_type=F32)
            ot_ref[pl.ds(vrow, HP), pl.ds(pl.multiple_of(qi * TQ, TQ), TQ)] = acc
            return c
        lax.fori_loop(0, NSTEP, fb, 0)

        def fin2(i, c):
            fin(i, False)
            out_cp(i).wait()
            return c
        lax.fori_loop(0, NFB, fin2, 0)


_SCRATCH = [
    pltpu.VMEM((S, D), BF16),
    pltpu.VMEM((D, D), BF16),
    pltpu.VMEM((D, D), BF16),
    pltpu.VMEM((D, D), BF16),
    pltpu.VMEM((D, D), BF16),
    pltpu.VMEM((D, DFF), BF16),
    pltpu.VMEM((DFF, D), BF16),
    pltpu.VMEM((S, D), BF16),
    pltpu.VMEM((2 * D, D), BF16),
    pltpu.VMEM((D // 2, DFF), F32),
    pltpu.VMEM((DFF // 2, D), F32),
    pltpu.VMEM((NT5, S, 128), F32),
    pltpu.VMEM((NSLAB, NLIMB, S // 4, 128), I32),
    pltpu.VMEM((NQ, D, TQ), F32),
    pltpu.VMEM((H * HP, S), F32),
    pltpu.VMEM((H * HP + HP, S), F32),
    pltpu.VMEM((S, D), F32),
    pltpu.VMEM((S, 128), F32),
    pltpu.VMEM((2 * S // 4, 128), I32),
    pltpu.VMEM((U * 32, TQ), I32),
    pltpu.VMEM((U * 8, TQ), F32),
] + [pltpu.VMEM((2 * NPER * HK, TQ), F32)] * NP + [
    pltpu.VMEM((D,), BF16),
    pltpu.SemaphoreType.DMA((7,)),
    pltpu.SemaphoreType.DMA((NB,)),
    pltpu.SemaphoreType.DMA((NFB,)),
]


@jax.jit
def pallas_gated_mix__softmax_full_mha__dense_activation_relu__prompt_kernel(
    A_x: jax.Array,
    A_wqkv: jax.Array,
    A_wo: jax.Array,
    B_x: jax.Array,
    B_w1: jax.Array,
    B_w2: jax.Array,
    gate_w: jax.Array,
):
    anyspec = pl.BlockSpec(memory_space=pl.ANY)
    out = pl.pallas_call(
        _kernel,
        out_shape=jax.ShapeDtypeStruct((S, D), BF16),
        in_specs=[anyspec] * 6,
        out_specs=anyspec,
        scratch_shapes=_SCRATCH,
        compiler_params=pltpu.CompilerParams(vmem_limit_bytes=100 * 1024 * 1024),
    )(A_x.reshape(S, D), A_wqkv, A_wo, B_w1, B_w2, gate_w)
    return out.reshape(1, S, D)
```
